```python
import os as _os
_os.environ.setdefault("JAX_PLATFORMS", "cpu")
import jax
import jax.numpy as jnp

def _softmax(x, axis=-1):
    return jax.nn.softmax(x, axis=axis)
def _gelu(x):
    return jax.nn.gelu(x, approximate=True)
def _silu(x):
    return jax.nn.silu(x)
def _sigmoid(x):
    return jax.nn.sigmoid(x)
def _layernorm(x, axis=-1, eps=1e-5):
    m = jnp.mean(x, axis=axis, keepdims=True)
    v = jnp.var(x, axis=axis, keepdims=True)
    return (x - m) / jnp.sqrt(v + eps)
def _scatter_add(tgt, idx, src, axis=0):
    return tgt.at[idx].add(src)
def _segment_sum(src, seg, n):
    return jax.ops.segment_sum(src, seg, n)
class _Rng:
    def __init__(self, key):
        self._k = key
    def _next(self):
        self._k, sub = jax.random.split(self._k)
        return sub
    def normal(self, shape):
        return jax.random.normal(self._next(), shape, dtype=jnp.bfloat16)
    def randint(self, lo, hi, shape):
        return jax.random.randint(self._next(), shape, lo, hi, dtype=jnp.int32)
    def uniform(self, shape, lo=0.0, hi=1.0):
        return jax.random.uniform(self._next(), shape, jnp.bfloat16, lo, hi)
    def permutation(self, n):
        return jax.random.permutation(self._next(), n)


kernel_name = 'sequential_preLN__ssm_conv_h3__mixer_channel_mlp__prompt'

def setup_inputs():
    _rng = _Rng(jax.random.key(int.from_bytes(__import__("os").urandom(4), "little")))
    _w = (lambda a: (lambda t: t.astype(jnp.bfloat16) if jnp.issubdtype(t.dtype, jnp.floating) else t)(jnp.asarray(a)))
    def _A_setup():
        B, S, D = 1, 2048, 448
        ks = 4
        return {
            "q": _w((lambda *s: _rng.normal(s) * 0.05)(B, S, D)),
            "k": _w((lambda *s: _rng.normal(s) * 0.05)(B, S, D)),
            "v": _w((lambda *s: _rng.normal(s) * 0.05)(B, S, D)),
            "shift_k": _w((lambda *s: _rng.normal(s) * 0.05)(D, ks) * 0.5),
            "ssm_k": _w((lambda *s: _rng.normal(s) * 0.05)(D, S) * (1.0 / S ** 0.5)),
            "ssm_D": _w((lambda *s: _rng.normal(s) * 0.05)(D)),
        }
    _A_in = _A_setup()

    def _B_setup():
        B, S, D, F = 1, 2048, 448, 1792
        return {
            "x": _w((lambda *s: _rng.normal(s) * 0.05)(B, S, D)),
            "w1": _w((lambda *s: _rng.normal(s) * 0.2)(D, F) * (D ** -0.5)),
            "b1": _w((lambda *s: _rng.normal(s) * 0.2)(F)),
            "w2": _w((lambda *s: _rng.normal(s) * 0.2)(F, D) * (F ** -0.5)),
            "b2": _w((lambda *s: _rng.normal(s) * 0.05)(D)),
        }
    _B_in = _B_setup()

    return {
        "A_q": _A_in["q"],
        "A_k": _A_in["k"],
        "A_v": _A_in["v"],
        "A_shift_k": _A_in["shift_k"],
        "A_ssm_k": _A_in["ssm_k"],
        "A_ssm_D": _A_in["ssm_D"],
        "B_x": _B_in["x"],
        "B_w1": _B_in["w1"],
        "B_b1": _B_in["b1"],
        "B_w2": _B_in["w2"],
        "B_b2": _B_in["b2"],
    }

def reference(A_q, A_k, A_v, A_shift_k, A_ssm_k, A_ssm_D, B_x, B_w1, B_b1, B_w2, B_b2):
    def _A_ref(q, k, v, shift_k, ssm_k, ssm_D):
        B, S, D = q.shape
        ks = shift_k.shape[-1]
        k_pad = jnp.pad(k, ((0, 0), (ks - 1, 0), (0, 0)))
        k_shift = jnp.zeros_like(k)
        for t in range(ks):
            k_shift = k_shift + k_pad[:, t:t + S, :] * shift_k[:, ks - 1 - t][None, None, :]
        kv = k_shift * v
        L = 2 * S
        kv_pad = jnp.pad(kv, ((0, 0), (0, S), (0, 0)))
        kf_pad = jnp.pad(ssm_k, ((0, 0), (0, S)))
        kv_f = (lambda x, axes=(-2,-1): jnp.fft.rfft2(x.astype(jnp.float32), axes=axes))(kv_pad[:, None, :, :], axes=(1, 2))
        kf_f = (lambda x, axes=(-2,-1): jnp.fft.rfft2(x.astype(jnp.float32), axes=axes))(kf_pad[:, None, :], axes=(1, 2))
        kf_f = (lambda x, *d: x.transpose(*d))(kf_f, 1, 2, 0)
        y_f = kv_f * kf_f[None, :, :, :]
        y = (lambda x, s, axes=(-2,-1): jnp.fft.irfft2(x, s=s, axes=axes).astype(jnp.bfloat16))(y_f, (1, L), axes=(1, 2))[:, 0, :S, :]
        y = y + kv * ssm_D[None, None, :]
        return q * y

    def _B_ref(x, w1, b1, w2, b2):
        y = _layernorm(x, axis=-1)
        h = _gelu(jnp.einsum("bsd,df->bsf", y, w1) + b1)
        return jnp.einsum("bsf,fd->bsd", h, w2) + b2

    x = A_q
    h = x + _A_ref(_layernorm(x, axis=-1), A_k, A_v, A_shift_k, A_ssm_k, A_ssm_D)
    h2 = h + _B_ref(_layernorm(h, axis=-1), B_w1, B_b1, B_w2, B_b2)
    return h2
```

```python
import numpy as np
import jax
import jax.numpy as jnp
import jax.experimental.pallas as pl
import jax.experimental.pallas.tpu as pltpu

S, D, F, KS = 2048, 448, 1792, 4
BL = 128
NB = S // BL
DP = 512
EPS = 1e-5
f32, bf16 = jnp.float32, jnp.bfloat16


def _dft_consts():
    t = np.arange(BL, dtype=np.float64)[:, None]
    f = np.arange(BL, dtype=np.float64)[None, :]
    th = 2.0 * np.pi * t * (f + 0.5) / (2 * BL)
    ft = np.concatenate([np.cos(th), -np.sin(th)], axis=1)
    gt = ft.T / BL
    return jnp.asarray(ft, dtype=bf16), jnp.asarray(gt, dtype=bf16)


def _gelu(x):
    c = 0.7978845608028654
    return 0.5 * x * (1.0 + jnp.tanh(c * (x + 0.044715 * (x * x * x))))


def _col(vec_row):
    return jnp.broadcast_to(vec_row, (128, D)).T


R = 64
TM = 256


def _kernel(q_ref, k_ref, v_ref, sk_ref, ssm_ref, d_ref, w1_ref, b1_ref, w2_ref, b2_ref,
            ft_ref, gt_ref, o_ref,
            cols_ref, w1t_ref, u_ref, kk_ref, yh_ref, y_ref):
    sk = sk_ref[...].astype(f32)
    for j in range(KS):
        cols_ref[j] = _col(sk[j:j + 1, :])
    cols_ref[4] = _col(d_ref[...].astype(f32).reshape(1, D))
    cols_ref[5] = _col(b2_ref[...].astype(f32).reshape(1, D))

    row = jax.lax.broadcasted_iota(jnp.int32, (DP - D, 128), 0)
    for j in range(F // 128):
        b1row = jnp.broadcast_to(b1_ref[j:j + 1, :].astype(f32), (DP - D, 128))
        tail = jnp.where(row == 0, b1row, 0.0)
        blk = jnp.concatenate([w1_ref[:, j * 128:(j + 1) * 128].astype(f32), tail], axis=0)
        w1t_ref[j * 128:(j + 1) * 128, :] = blk.T.astype(bf16)

    lane = jax.lax.broadcasted_iota(jnp.int32, (R, 128), 1)
    sgn = jnp.where((lane & 1) == 0, 1.0, -1.0).astype(f32)

    def conv_group(g, carry):
        r0 = pl.multiple_of(g * R, R)
        rows = pl.ds(r0, R)
        kf = k_ref[rows, :].astype(f32)
        ksh = kf * jnp.tile(cols_ref[0, rows, :], (1, NB))
        for j in range(1, KS):
            rj = pltpu.roll(kf, j, 1)
            rj = jnp.concatenate([jnp.where(lane < j, 0.0, rj[:, :128]), rj[:, 128:]], axis=1)
            ksh = ksh + rj * jnp.tile(cols_ref[j, rows, :], (1, NB))
        kv = (ksh * v_ref[rows, :].astype(f32)).astype(bf16)
        ssm = ssm_ref[rows, :]
        lhs = jnp.concatenate([kv[:, a * BL:(a + 1) * BL] for a in range(NB)]
                              + [ssm[:, a * BL:(a + 1) * BL] for a in range(NB)], axis=0)
        spec = jnp.dot(lhs, ft_ref[...], preferred_element_type=f32)
        for a in range(NB):
            ur = spec[a * R:(a + 1) * R, :128]
            ui = spec[a * R:(a + 1) * R, 128:]
            u_ref[0, a] = ur + ui
            u_ref[1, a] = ur
            u_ref[2, a] = ui
        dcol = cols_ref[4, rows, :]
        for a in range(NB):
            p = spec[(NB + a) * R:(NB + a + 1) * R, :128]
            q = spec[(NB + a) * R:(NB + a + 1) * R, 128:]
            if a == 0:
                c = p + dcol
                d = q
            else:
                pp = spec[(NB + a - 1) * R:(NB + a) * R, :128]
                qq = spec[(NB + a - 1) * R:(NB + a) * R, 128:]
                c = p - sgn * qq
                d = q + sgn * pp
            kk_ref[0, a] = c
            kk_ref[1, a] = d - c
            kk_ref[2, a] = c + d

        def mac(p, carry2):
            rr = pl.ds(pl.multiple_of(p * 8, 8), 8)
            us = [u_ref[0, a, rr, :] for a in range(NB)]
            ks = [kk_ref[0, a, rr, :] for a in range(NB)]
            s1 = []
            for a in range(NB):
                acc = us[0] * ks[a]
                for b in range(1, a + 1):
                    acc = acc + us[b] * ks[a - b]
                s1.append(acc)
            us = [u_ref[2, a, rr, :] for a in range(NB)]
            ks = [kk_ref[2, a, rr, :] for a in range(NB)]
            for a in range(NB):
                acc = s1[a]
                for b in range(a + 1):
                    acc = acc - us[b] * ks[a - b]
                yh_ref[a, rr, 0:128] = acc
            us = [u_ref[1, a, rr, :] for a in range(NB)]
            ks = [kk_ref[1, a, rr, :] for a in range(NB)]
            for a in range(NB):
                acc = s1[a]
                for b in range(a + 1):
                    acc = acc + us[b] * ks[a - b]
                yh_ref[a, rr, 128:256] = acc
            return carry2
        jax.lax.fori_loop(0, R // 8, mac, 0)

        yh = yh_ref[...].reshape(NB * R, 256).astype(bf16)
        y = jnp.dot(yh, gt_ref[...], preferred_element_type=f32)
        for a in range(NB):
            y_ref[rows, a * BL:(a + 1) * BL] = y[a * R:(a + 1) * R, :]
        return carry
    jax.lax.fori_loop(0, D // R, conv_group, 0)

    rowt = jax.lax.broadcasted_iota(jnp.int32, (DP - D, TM), 0)
    ones_tail = jnp.where(rowt == 0, 1.0, 0.0).astype(bf16)

    def mlp_tile(t, carry):
        cs = pl.ds(pl.multiple_of(t * TM, TM), TM)
        x = q_ref[:, cs].astype(f32)
        m = jnp.mean(x, axis=0, keepdims=True)
        xc = x - m
        var = jnp.mean(xc * xc, axis=0, keepdims=True)
        qn = xc * jax.lax.rsqrt(var + EPS)
        h = x + qn * y_ref[:, cs]
        m1 = jnp.mean(h, axis=0, keepdims=True)
        hc = h - m1
        v1 = jnp.mean(hc * hc, axis=0, keepdims=True)
        z = hc * jax.lax.rsqrt(v1 + EPS)
        m2 = jnp.mean(z, axis=0, keepdims=True)
        zc = z - m2
        v2 = jnp.mean(zc * zc, axis=0, keepdims=True)
        zn = (zc * jax.lax.rsqrt(v2 + EPS)).astype(bf16)
        xa = jnp.concatenate([zn, ones_tail], axis=0)
        pre = jnp.dot(w1t_ref[...], xa, preferred_element_type=f32)
        g = _gelu(pre).astype(bf16)
        out = jnp.dot(w2_ref[...], g, preferred_element_type=f32)
        out = out + h + jnp.tile(cols_ref[5], (1, TM // 128))
        o_ref[:, cs] = out.astype(o_ref.dtype)
        return carry
    jax.lax.fori_loop(0, S // TM, mlp_tile, 0)


@jax.jit
def pallas_sequential_preLN__ssm_conv_h3__mixer_channel_mlp__prompt_kernel(
    A_q, A_k, A_v, A_shift_k, A_ssm_k, A_ssm_D, B_x, B_w1, B_b1, B_w2, B_b2,
):
    ft, gt = _dft_consts()
    outT = pl.pallas_call(
        _kernel,
        out_shape=jax.ShapeDtypeStruct((D, S), bf16),
        scratch_shapes=[
            pltpu.VMEM((6, D, 128), f32),
            pltpu.VMEM((F, DP), bf16),
            pltpu.VMEM((3, NB, R, 128), f32),
            pltpu.VMEM((3, NB, R, 128), f32),
            pltpu.VMEM((NB, R, 256), f32),
            pltpu.VMEM((D, S), f32),
        ],
        compiler_params=pltpu.CompilerParams(vmem_limit_bytes=100 * 1024 * 1024),
    )(A_q[0].T, A_k[0].T, A_v[0].T, A_shift_k.T, A_ssm_k, A_ssm_D, B_w1,
      B_b1.reshape(F // 128, 128), B_w2.T, B_b2, ft, gt)
    return outT.T[None]
```

```python
import os
import numpy as np
import jax
import jax.numpy as jnp
import jax.experimental.pallas as pl
import jax.experimental.pallas.tpu as pltpu

S, D, F, KS = 2048, 448, 1792, 4
BL = 128
NB = S // BL
DP = 512
EPS = 1e-5
TM = 256
NT = S // TM
BPT = TM // BL
FC = 256
NFC = F // FC
SPC = FC // 128
LSTEP = int(os.environ.get('LSTEP', 8))
NP = D // 8
RG = int(os.environ.get('RG', 64))
f32, bf16, u32 = jnp.float32, jnp.bfloat16, jnp.uint32

KV_TIE = int(os.environ.get('KV_TIE', 4))
DFT_BACK = int(os.environ.get('DFT_BACK', 1))
L_DFT = float(os.environ.get('L_DFT', 14.0))

SEM_G = 0
SEM_H = 12
SEM_O = 16
NSEM = 17
AK, AV, AQ = 0, 1, 2


def _pack_np(a):
    u = np.ascontiguousarray(a, dtype=np.float32).view(np.uint32)
    b = (u + 0x7FFF + ((u >> 16) & 1)) >> 16
    return (b[..., 0::2, :] | (b[..., 1::2, :] << 16)).astype(np.uint32)


def _dft_consts():
    t = np.arange(BL, dtype=np.float64)[:, None]
    f = np.arange(BL, dtype=np.float64)[None, :]
    th = 2.0 * np.pi * t * (f + 0.5) / (2 * BL)
    ft = np.stack([np.cos(th), -np.sin(th)], axis=0)
    gt = np.concatenate([np.cos(th).T, -np.sin(th).T], axis=0) / BL
    return jnp.asarray(_pack_np(ft)), jnp.asarray(_pack_np(gt))


def _gelu2(x):
    c = 0.7978845608028654
    return x * (1.0 + jnp.tanh(x * (c + (c * 0.044715) * (x * x))))


def _col(vec_row):
    return jnp.broadcast_to(vec_row, (128, D)).T


def _pk(x):
    return pltpu.bitcast(x, u32)


def _upk(x):
    return pltpu.bitcast(x, bf16)


def _pack2(a, b):
    return pltpu.bitcast(pltpu.pack_elementwise([a, b], packed_dtype=bf16), u32)


def _pack_groups(x):
    n = x.shape[0] // 16
    return jnp.concatenate([_pack2(x[16 * m:16 * m + 8], x[16 * m + 8:16 * m + 16]) for m in range(n)], axis=0)


def _rowsum8(x, tie=None):
    n = x.shape[0] // 8
    acc = x[0:8] if tie is None else tie(x[0:8])
    for i in range(1, n):
        acc = acc + x[i * 8:(i + 1) * 8]
    return acc


def _mean8(acc8):
    return jnp.broadcast_to(jnp.sum(acc8, axis=0, keepdims=True) * (1.0 / D), (8, 128))


def _tile8(stat8, n):
    return jnp.concatenate([stat8] * (n // 8), axis=0)


def _kernel(q_hbm, k_hbm, v_hbm, sk_hbm, ssm_hbm, d_hbm, w1_hbm, b1_hbm, w2_hbm, b2_hbm,
            ft_hbm, gt_hbm, o_hbm,
            q_ref, k_ref, v_ref, sk_ref, ssm_ref, d_ref, w1_ref, b1_ref, w2_ref, b2_ref,
            ft_ref, gt_ref, o_ref,
            cols_ref, w1t_ref, uk_ref, kraw_ref, yh_ref, kv_ref, h_ref, xa_ref, acc_ref,
            st_ref, g_ref, w2p_ref, tmp_ref, sems):
    def col_slice(i, w):
        if isinstance(i, int):
            return pl.ds(i * w, w)
        return pl.ds(pl.multiple_of(i * w, w), w)

    def cp(src, dst, sem):
        return pltpu.make_async_copy(src, dst, sems.at[sem])

    def q_in(t, sem):
        return [cp(q_hbm.at[:, col_slice(t, TM)], q_ref.at[t], sem)]

    def tile_in(t, sem, sem2=None):
        sem2 = sem if sem2 is None else sem2
        return ([cp(k_hbm.at[:, col_slice(t, TM)], k_ref.at[t], sem),
                 cp(v_hbm.at[:, col_slice(t, TM)], v_ref.at[t], sem)]
                + [cp(ssm_hbm.at[:, col_slice(t * BPT + a, BL)], ssm_ref.at[t * BPT + a], sem2) for a in range(BPT)])

    def w1_in(c0, c1, sem):
        sl = pl.ds(c0 * FC, (c1 - c0) * FC)
        return [cp(w1_hbm.at[:, sl], w1_ref.at[:, sl], sem)]

    def w2_in(c0, c1, sem):
        return [cp(w2_hbm.at[:, col_slice(j, 128)], w2_ref.at[j], sem) for j in range(c0 * SPC, c1 * SPC)]

    def out_cp(t, sem):
        return [cp(o_ref.at[t * BPT + a], o_hbm.at[:, col_slice(t * BPT + a, BL)], sem) for a in range(BPT)]

    t0 = tile_in(0, SEM_G + 1, SEM_G + 2)
    G = [
        [cp(s, d, SEM_G) for s, d in [(sk_hbm, sk_ref), (d_hbm, d_ref), (b2_hbm, b2_ref), (b1_hbm, b1_ref)]],
        t0[:2],
        [cp(ft_hbm, ft_ref, SEM_G + 2)] + t0[2:],
        [cp(gt_hbm, gt_ref, SEM_G + 3)] + q_in(0, SEM_G + 3),
        w1_in(0, 3, SEM_G + 4),
        w1_in(3, 7, SEM_G + 5),
        tile_in(1, SEM_G + 6) + q_in(1, SEM_G + 6),
        w2_in(0, 4, SEM_G + 7),
        w2_in(4, 7, SEM_G + 8) + tile_in(2, SEM_G + 8),
        q_in(2, SEM_G + 9) + tile_in(3, SEM_G + 9),
        tile_in(4, SEM_G + 10),
        q_in(3, SEM_G + 11),
    ]
    H = [q_in(t + 2, SEM_H + t - 2) + (tile_in(t + 3, SEM_H + t - 2) if t + 3 < NT else []) for t in range(2, NT - 2)]
    for grp in G + H:
        for c in grp:
            c.start()

    def wait(copies):
        for c in copies:
            c.wait()

    def prep_cols():
        def init(i, c):
            z8 = jnp.zeros((8, 128), f32)
            zu = jnp.zeros((8, 128), u32)
            uk_ref[0, i, 0] = z8
            kraw_ref[i, 0:8, :] = z8
            st_ref[i, 0] = z8
            g_ref[i, 0, 0:8, :] = zu
            w2p_ref[i, 0:8, :] = zu
            w1t_ref[i, 0:8, :] = zu
            tmp_ref[i, 0, 0:8, :] = z8
            cols_ref[i, 0:8, :] = z8
            yh_ref[i, 0, 0:16, :] = jnp.zeros((16, 128), bf16)
            kv_ref[pl.ds(pl.multiple_of(i * 8, 8), 8), :] = zu
            return c
        jax.lax.fori_loop(0, 2, init, 0)
        sk = sk_ref[...].astype(f32)
        for j in range(KS):
            cols_ref[j] = _col(sk[j:j + 1, :])

    def prep_more():
        cols_ref[4] = _col(d_ref[...].astype(f32).reshape(1, D))
        cols_ref[5] = _col(b2_ref[...].astype(f32).reshape(1, D))
        rowt = jax.lax.broadcasted_iota(jnp.int32, (DP - D, 128), 0)
        tail = jnp.where(rowt == 0, 1.0, 0.0).astype(bf16)
        for par in range(2):
            for b in range(BPT):
                xa_ref[par, b, D // 2:DP // 2, :] = _pk(tail)

    def w1t_gen(c0, c1):
        row = jax.lax.broadcasted_iota(jnp.int32, (DP - D, 128), 0)
        for j in range(c0 * SPC, c1 * SPC):
            for kt in range(DP // 128):
                tie = yield
                r0, r1 = kt * 128, min((kt + 1) * 128, D)
                w = w1_ref[r0:r1, j * 128:(j + 1) * 128].astype(f32)
                w = jnp.concatenate([w[:-8], tie(w[-8:])], axis=0)
                blk = _upk(_pack_groups(w)).astype(f32)
                if r1 - r0 < 128:
                    b1row = jnp.broadcast_to(b1_ref[j:j + 1, :].astype(f32), (DP - D, 128))
                    blk = jnp.concatenate([blk, jnp.where(row == 0, b1row, 0.0)], axis=0)
                tmp_ref[j, kt] = blk.T
                for m in range(4):
                    rows = [tmp_ref[j, kt, pl.ds(32 * m + o, 8, stride=4), :] for o in range(4)]
                    base = j * 64 + m * 16
                    w1t_ref[kt, base:base + 8, :] = _pack2(rows[0], rows[2])
                    w1t_ref[kt, base + 8:base + 16, :] = _pack2(rows[1], rows[3])

    def w1t_units(c0, c1):
        return (c1 - c0) * SPC * (DP // 128)

    def put(slot, sub, val):
        uk_ref[slot, :, sub] = val.reshape(NP, 8, 128)

    def kv_gen(t):
        def halves(w):
            return (pltpu.bitcast(w << 16, f32), pltpu.bitcast(w & jnp.uint32(0xFFFF0000), f32))
        for r0 in range(0, D, 16):
            tie = yield
            r1 = r0 + 16
            kc = [_pk(k_ref[t, r0:r1, a * BL:(a + 1) * BL]) for a in range(BPT)]
            prev = jnp.zeros((8, 128), u32) if t == 0 else _pk(k_ref[t - 1, r0:r1, TM - 128:TM])
            kf = jnp.concatenate([prev] + kc, axis=1)
            if KV_TIE & 1:
                kf = pltpu.bitcast(jnp.concatenate(
                    [tie(pltpu.bitcast(kf[:, i * 128:(i + 1) * 128], f32)) for i in range(BPT + 1)], axis=1), u32)
            sh = [kf[:, 128:]] + [pltpu.roll(kf, j, 1)[:, 128:] for j in range(1, KS)]
            vw = jnp.concatenate([_pk(v_ref[t, r0:r1, a * BL:(a + 1) * BL]) for a in range(BPT)], axis=1)
            res = []
            for o in range(2):
                acc = None
                for j in range(KS):
                    cj = cols_ref[j, pl.ds(r0 + o, 8, stride=2), :]
                    if j == 0 and KV_TIE & 4:
                        cj = tie(cj)
                    cj = jnp.tile(cj, (1, BPT))
                    term = halves(sh[j])[o] * cj
                    acc = term if acc is None else acc + term
                res.append(acc * halves(vw)[o])
            for a in range(BPT):
                cs = slice(a * BL, (a + 1) * BL)
                pk = _pack2(res[0][:, cs], res[1][:, cs])
                if KV_TIE & 2:
                    pk = pltpu.bitcast(tie(pltpu.bitcast(pk, f32)), u32)
                kv_ref[(a * D + r0) // 2:(a * D + r1) // 2, :] = pk

    KV_UNITS = D // 16

    def dft(t):
        lane = jax.lax.broadcasted_iota(jnp.int32, (16, 128), 1)
        sgn = jnp.where((lane & 1) == 0, 1.0, -1.0).astype(f32)
        ft = jnp.concatenate([_upk(ft_ref[0]), _upk(ft_ref[1])], axis=1)
        lk = jnp.concatenate([ssm_ref[t * BPT + a, r0:r0 + 16, :] for r0 in range(0, D, 16) for a in range(BPT)],
                             axis=0)
        sk_ = jnp.dot(lk, ft, preferred_element_type=f32)
        su = jnp.dot(_upk(kv_ref[...]), ft, preferred_element_type=f32)
        for r0 in range(0, D, 16):
            ps = slice(r0 // 8, r0 // 8 + 2)
            for a in range(BPT):
                blk = t * BPT + a
                o = BPT * r0 + 16 * a
                p = sk_[o:o + 16, :128]
                q = sk_[o:o + 16, 128:]
                if blk == 0:
                    c = p + cols_ref[4, r0:r0 + 16, :]
                    d = q
                else:
                    if a == 0:
                        pp = kraw_ref[0, r0:r0 + 16, :]
                        qq = kraw_ref[1, r0:r0 + 16, :]
                    c = p - qq
                    d = q + pp
                uk_ref[blk, ps, 3] = c.reshape(2, 8, 128)
                uk_ref[blk, ps, 4] = (d - c).reshape(2, 8, 128)
                uk_ref[blk, ps, 5] = (c + d).reshape(2, 8, 128)
                if blk < NB - 1:
                    pp = sgn * p
                    qq = sgn * q
                    if a == BPT - 1:
                        kraw_ref[0, r0:r0 + 16, :] = pp
                        kraw_ref[1, r0:r0 + 16, :] = qq
        for a in range(BPT):
            ur = su[a * D:(a + 1) * D, :128]
            ui = su[a * D:(a + 1) * D, 128:]
            blk = t * BPT + a + 1
            put(blk, 0, ur + ui)
            put(blk, 1, ur)
            put(blk, 2, ui)
        return su

    def mac_gen(t, nlag, tmin=None):
        static = isinstance(t, int)
        a_last = t * BPT + BPT - 1
        if static:
            uslot = [max(a_last - e + 1, 0) for e in range(nlag)]
            kslot = [min(dl, a_last) for dl in range(nlag)]
        else:
            amin = tmin * BPT + BPT - 1
            uslot = [jnp.maximum(a_last - e + 1, 0) if amin - e + 1 < 0 else a_last - e + 1 for e in range(nlag)]
            kslot = [jnp.minimum(dl, a_last) if dl > amin else dl for dl in range(nlag)]
        for p in range(NP):
            if p % 2 == 0:
                re_rows = [[] for _ in range(BPT)]
                im_rows = [[] for _ in range(BPT)]
            res = [None] * BPT
            for comp, sign in ((0, 1), (2, -1), (1, 1)):
                accs = [None] * BPT if comp == 0 else list(res)
                us = {}
                for l0 in range(0, nlag, LSTEP):
                    tie = yield
                    l1 = min(l0 + LSTEP, nlag)
                    for dl in range(l0, l1):
                        kx = uk_ref[kslot[dl], p, 3 + comp]
                        if dl == l0:
                            kx = tie(kx)
                        for i in range(BPT):
                            e = dl + BPT - 1 - i
                            if e >= nlag:
                                continue
                            if e not in us:
                                us[e] = uk_ref[uslot[e], p, comp]
                            pr = us[e] * kx
                            if accs[i] is None:
                                accs[i] = pr
                            elif sign > 0:
                                accs[i] = accs[i] + pr
                            else:
                                accs[i] = accs[i] - pr
                for i in range(BPT):
                    if comp == 0:
                        res[i] = accs[i]
                    elif comp == 2:
                        re_rows[i].append(accs[i])
                    else:
                        im_rows[i].append(accs[i])
            if p % 2 == 1:
                rr = slice((p // 2) * 16, (p // 2) * 16 + 16)
                for i in range(BPT):
                    yh_ref[i, 0, rr, :] = jnp.concatenate(re_rows[i], axis=0).astype(bf16)
                    yh_ref[i, 1, rr, :] = jnp.concatenate(im_rows[i], axis=0).astype(bf16)

    def mac_units(nlag):
        return NP * 3 * (-(-nlag // LSTEP))

    def inv(b):
        yh = jnp.concatenate([yh_ref[b, 0], yh_ref[b, 1]], axis=1)
        return jnp.dot(yh, _upk(gt_ref[...]), preferred_element_type=f32)

    def xstats_gen(t):
        for b in range(BPT):
            cs = slice(b * BL, (b + 1) * BL)
            acc = None
            for r0 in range(0, D, RG):
                tie = yield
                s = _rowsum8(q_ref[t, r0:r0 + RG, cs].astype(f32), tie)
                acc = s if acc is None else acc + s
            st_ref[b, 0] = _mean8(acc)
        for b in range(BPT):
            cs = slice(b * BL, (b + 1) * BL)
            acc = None
            for r0 in range(0, D, RG):
                tie = yield
                xc = q_ref[t, r0:r0 + RG, cs].astype(f32) - _tile8(tie(st_ref[b, 0]), RG)
                s = _rowsum8(xc * xc)
                acc = s if acc is None else acc + s
            st_ref[b, 1] = jax.lax.rsqrt(_mean8(acc) + EPS)

    XSTAT_UNITS = 2 * BPT * (D // RG)

    def pass_c(t, par, b, y):
        cs = slice(b * BL, (b + 1) * BL)
        x = q_ref[t, :, cs].astype(f32)
        xc = x - _tile8(st_ref[b, 0], D)
        h = x + xc * (y * _tile8(st_ref[b, 1], D))
        h_ref[par, b] = h
        return _mean8(_rowsum8(h))

    def hln_gen(par, m1):
        r1 = [None] * BPT
        m2 = [None] * BPT
        r2 = [None] * BPT
        for b in range(BPT):
            acc = None
            for r0 in range(0, D, RG):
                tie = yield
                hc = h_ref[par, b, r0:r0 + RG, :] - _tile8(tie(m1[b]), RG)
                s = _rowsum8(hc * hc)
                acc = s if acc is None else acc + s
            r1[b] = jax.lax.rsqrt(_mean8(acc) + EPS)
        for b in range(BPT):
            acc = None
            for r0 in range(0, D, RG):
                tie = yield
                zz = (h_ref[par, b, r0:r0 + RG, :] - _tile8(tie(m1[b]), RG)) * _tile8(r1[b], RG)
                s = _rowsum8(zz)
                acc = s if acc is None else acc + s
            m2[b] = _mean8(acc)
        for b in range(BPT):
            acc = None
            for r0 in range(0, D, RG):
                tie = yield
                zc = (h_ref[par, b, r0:r0 + RG, :] - _tile8(tie(m1[b]), RG)) * _tile8(r1[b], RG) - _tile8(m2[b], RG)
                s = _rowsum8(zc * zc)
                acc = s if acc is None else acc + s
            r2[b] = jax.lax.rsqrt(_mean8(acc) + EPS)
        for b in range(BPT):
            for r0 in range(0, D, RG):
                tie = yield
                zc = (h_ref[par, b, r0:r0 + RG, :] - _tile8(tie(m1[b]), RG)) * _tile8(r1[b], RG) - _tile8(m2[b], RG)
                xa_ref[par, b, r0 // 2:(r0 + RG) // 2, :] = _pack_groups(zc * _tile8(r2[b], RG))

    HLN_UNITS = 4 * BPT * (D // RG)

    def run_all(gen):
        next(gen)
        while True:
            try:
                gen.send(lambda x: x)
            except StopIteration:
                return

    NCAND = {'mm1': 64, 'mm2': 56, 'inv': 56, 'dft': 112}
    LOAD = {'mm1': 10.0, 'mm2': 4.5, 'inv': 18.0, 'dft': L_DFT}

    def s_mac(t, p0, p1):
        nlag = BPT * (t + 1)
        n = mac_units(nlag)
        return (lambda: mac_gen(t, nlag), n, (NP * 6.0 * (2 * nlag - 1) + 340) / n + 1, p0, p1)

    def s_hln(par, p0, p1):
        return (lambda: hln_gen(par, state['m1']), HLN_UNITS, 34.0, p0, p1)

    def s_xs(t, p0, p1):
        return (lambda: xstats_gen(t), XSTAT_UNITS, 26.0, p0, p1)

    def s_kv(t, p0, p1):
        return (lambda: kv_gen(t), KV_UNITS, 70.0, p0, p1)

    def s_w1t(c0, c1, p0, p1):
        return (lambda: w1t_gen(c0, c1), w1t_units(c0, c1), 60.0, p0, p1)

    state = {}

    def segment(phases, streams):
        always = gt_ref[0:8, :] != jnp.uint32(0x7FC17FC1)
        pos, load, keys = [], [], []
        for pi, ph in enumerate(phases):
            n = NCAND.get(ph[0], 0)
            for c in range(n):
                pos.append(pi + (c + 0.5) / n)
                load.append(LOAD[ph[0]])
                keys.append((pi, c))
        pos, load = np.array(pos), np.array(load, dtype=np.float64)
        plan = {}
        for si, (mk, n, cost, p0, p1) in enumerate(streams):
            idx = np.nonzero((pos >= p0) & (pos <= p1))[0]
            lo, hi = 0.0, 1000.0
            for _ in range(60):
                mid = 0.5 * (lo + hi)
                if np.maximum(mid - load[idx], 0).sum() < n * cost:
                    lo = mid
                else:
                    hi = mid
            add = np.maximum(hi - load[idx], 0) + 1e-9
            load[idx] += add
            if os.environ.get('SHOW_LOAD'):
                print('stream', si, 'units', n, 'level', round(hi / 8, 2))
            cums = np.cumsum(add) / add.sum()
            holder = {}

            def fire(val, mk=mk, holder=holder):
                if 'g' not in holder:
                    holder['g'] = mk()
                    next(holder['g'])
                try:
                    holder['g'].send(lambda x: jnp.where(always, x, val))
                except StopIteration:
                    pass
            for u in range(n):
                ci = idx[min(int(np.searchsorted(cums, (u + 0.5) / n)), len(idx) - 1)]
                plan.setdefault(keys[ci], []).append(fire)

        def fire_all(pi, getter):
            for c in range(NCAND[phases[pi][0]]):
                for fire in plan.get((pi, c), []):
                    fire(getter(c))

        for pi, ph in enumerate(phases):
            kind = ph[0]
            if kind == 'mm1':
                _, par, j = ph
                xa = jnp.concatenate([_upk(xa_ref[par, b]) for b in range(BPT)], axis=1)
                w1c = jnp.concatenate([_upk(w1t_ref[kt, j * FC // 2:(j + 1) * FC // 2, :])
                                       for kt in range(DP // 128)], axis=1)
                pre = jnp.dot(w1c, xa, preferred_element_type=f32)
                g = _gelu2(pre)
                for b in range(BPT):
                    gb = g[:, b * BL:(b + 1) * BL]
                    for m in range(FC // 32):
                        r = 32 * m
                        g_ref[j, b, 16 * m:16 * m + 8, :] = _pack2(gb[r:r + 8], gb[r + 16:r + 24])
                        g_ref[j, b, 16 * m + 8:16 * m + 16, :] = _pack2(gb[r + 8:r + 16], gb[r + 24:r + 32])
                fire_all(pi, lambda c: pre[(c % 32) * 8:(c % 32) * 8 + 8, (c // 32) * 128:(c // 32) * 128 + 128])
            elif kind == 'mm2':
                _, j, raw = ph
                if raw:
                    slabs = [w2_ref[j * SPC + kt] for kt in range(SPC)]
                    for kt in range(SPC):
                        w2p_ref[j * SPC + kt] = _pk(slabs[kt])
                else:
                    slabs = [_upk(w2p_ref[j * SPC + kt]) for kt in range(SPC)]
                gj = jnp.concatenate([_upk(g_ref[j, b]) for b in range(BPT)], axis=1)
                part = jnp.dot(jnp.concatenate(slabs, axis=1), gj, preferred_element_type=f32)
                state['acc'] = part if j == 0 else state['acc'] + part
                fire_all(pi, lambda c: part[c * 8:c * 8 + 8, 0:128])
            elif kind == 'inv':
                _, t, par = ph
                ys = [inv(b) for b in range(BPT)]
                state['m1'] = [pass_c(t, par, b, ys[b]) for b in range(BPT)]
                fire_all(pi, lambda c: ys[0][c * 8:c * 8 + 8, :])
            elif kind == 'dft':
                _, t = ph
                su = dft(t)
                fire_all(pi, lambda c: su[c * 8:c * 8 + 8, 0:128])
            elif kind == 'out':
                _, t, par = ph
                acc = state['acc']
                for b in range(BPT):
                    o_ref[t * BPT + b] = (0.5 * acc[:, b * BL:(b + 1) * BL]
                                          + (h_ref[par, b] + cols_ref[5])).astype(o_ref.dtype)
            elif kind == 'acc_store':
                acc_ref[...] = state['acc']
            elif kind == 'acc_load':
                state['acc'] = acc_ref[...]
            elif kind == 'send':
                _, t, sem = ph
                for c in out_cp(t, sem):
                    c.start()

    def mlp_phases(par, j0, j1):
        ph = []
        for j in range(j0, j1):
            if j < NFC:
                ph.append(('mm1', par, j))
            if j > 0:
                ph.append(('mm2', j - 1, False))
        return ph

    def steady(t, sem_out):
        par = t % 2
        do_ln = t + 1 < NT
        phases = ([('inv', t + 1, 1 - par)] if do_ln else []) + mlp_phases(par, 0, NFC + 1)
        streams = []
        if t + 3 < NT:
            pd = len(phases) - DFT_BACK
            phases.insert(pd, ('dft', t + 3))
            streams.append(s_kv(t + 3, 1.0, pd - 0.5))
        end = len(phases) - 0.4
        if do_ln:
            streams.append(s_hln(1 - par, 1.3, end))
        if t + 2 < NT:
            streams.append(s_xs(t + 2, 1.3, end))
            streams.append(s_mac(t + 2, 1.0, end))
        phases += [('out', t, par), ('send', t, sem_out)]
        segment(phases, streams)

    wait(G[0])
    prep_cols()
    wait(G[1])
    run_all(kv_gen(0))
    prep_more()
    wait(G[2])
    dft(0)
    wait(G[3])
    run_all(mac_gen(0, BPT))
    run_all(xstats_gen(0))
    m1_0 = [pass_c(0, 0, b, inv(b)) for b in range(BPT)]
    wait(G[4])
    run_all(hln_gen(0, m1_0))
    run_all(w1t_gen(0, 2))
    segment([('mm1', 0, 0), ('mm1', 0, 1)], [s_w1t(2, 3, 0.2, 1.5)])
    wait(G[5])
    segment([('mm1', 0, 2), ('mm1', 0, 3), ('mm1', 0, 4)],
            [s_w1t(3, 4, 0.0, 0.6), s_w1t(4, 5, 0.5, 1.4), s_w1t(5, 7, 1.3, 2.5)])
    wait(G[6])
    segment([('mm1', 0, 5), ('mm1', 0, 6), ('dft', 1)], [s_kv(1, 0.0, 1.8), s_xs(1, 1.8, 2.7)])
    wait(G[7])
    segment([('mm2', j, True) for j in range(4)], [s_mac(1, 0.0, 3.7)])
    wait(G[8])
    segment([('inv', 1, 1)] + [('mm2', j, True) for j in range(4, 7)] + [('out', 0, 0), ('send', 0, SEM_O)],
            [s_hln(1, 1.2, 3.7), s_kv(2, 0.3, 3.7)])
    wait(G[9])
    segment([('dft', 2), ('mm1', 1, 0), ('mm1', 1, 1)], [s_kv(3, 1.0, 2.7), s_xs(2, 0.0, 2.7)])
    wait(G[10])
    segment([('dft', 3), ('mm2', 0, False)] + mlp_phases(1, 2, 4), [s_kv(4, 1.0, 5.6), s_mac(2, 0.0, 5.6)])
    wait(G[11])
    segment([('inv', 2, 0), ('dft', 4)] + mlp_phases(1, 4, 8) + [('out', 1, 1), ('send', 1, SEM_O)],
            [s_hln(0, 1.3, 8.6), s_xs(3, 1.3, 8.6), s_mac(3, 1.0, 8.6)])
    for t in range(2, 6):
        wait(H[t - 2])
        steady(t, SEM_O)

    JS = 3

    def tail(i, carry):
        @pl.when(i == 0)
        def _():
            segment([('inv', 7, 1)] + mlp_phases(0, 0, JS) + [('acc_store',)], [s_hln(1, 1.3, 2 * JS - 0.4)])

        @pl.when(i == 1)
        def _():
            segment(mlp_phases(1, 0, JS) + [('acc_store',)], [])
        segment([('acc_load',)] + mlp_phases(i, JS, NFC + 1) + [('out', 6 + i, i), ('send', 6 + i, SEM_O)], [])
        return carry
    jax.lax.fori_loop(0, 2, tail, 0)
    for t in range(NT):
        wait(out_cp(t, SEM_O))


@jax.jit
def pallas_sequential_preLN__ssm_conv_h3__mixer_channel_mlp__prompt_kernel(
    A_q, A_k, A_v, A_shift_k, A_ssm_k, A_ssm_D, B_x, B_w1, B_b1, B_w2, B_b2,
):
    ft, gt = _dft_consts()
    any_spec = pl.BlockSpec(memory_space=pl.ANY)
    outT = pl.pallas_call(
        _kernel,
        out_shape=jax.ShapeDtypeStruct((D, S), bf16),
        in_specs=[any_spec] * 12,
        out_specs=any_spec,
        scratch_shapes=[
            pltpu.VMEM((NT, D, TM), bf16),
            pltpu.VMEM((NT, D, TM), bf16),
            pltpu.VMEM((NT, D, TM), bf16),
            pltpu.VMEM((KS, D), bf16),
            pltpu.VMEM((NB, D, BL), bf16),
            pltpu.VMEM((D,), bf16),
            pltpu.VMEM((D, F), bf16),
            pltpu.VMEM((F // 128, 128), bf16),
            pltpu.VMEM((F // 128, D, 128), bf16),
            pltpu.VMEM((D,), bf16),
            pltpu.VMEM((2, BL // 2, BL), u32),
            pltpu.VMEM((BL, BL), u32),
            pltpu.VMEM((NB, D, BL), bf16),
            pltpu.VMEM((6, D, 128), f32),
            pltpu.VMEM((DP // 128, F // 2, 128), u32),
            pltpu.VMEM((NB + 1, NP, 6, 8, 128), f32),
            pltpu.VMEM((2, D, 128), f32),
            pltpu.VMEM((BPT, 2, D, 128), bf16),
            pltpu.VMEM((BPT * D // 2, 128), u32),
            pltpu.VMEM((2, BPT, D, BL), f32),
            pltpu.VMEM((2, BPT, DP // 2, BL), u32),
            pltpu.VMEM((D, TM), f32),
            pltpu.VMEM((BPT, 2, 8, 128), f32),
            pltpu.VMEM((NFC, BPT, FC // 2, BL), u32),
            pltpu.VMEM((F // 128, D // 2, 128), u32),
            pltpu.VMEM((F // 128, DP // 128, 128, 128), f32),
            pltpu.SemaphoreType.DMA((NSEM,)),
        ],
        compiler_params=pltpu.CompilerParams(vmem_limit_bytes=110 * 1024 * 1024),
    )(A_q[0].T, A_k[0].T, A_v[0].T, A_shift_k.T, A_ssm_k, A_ssm_D, B_w1,
      B_b1.reshape(F // 128, 128), B_w2.T, B_b2, ft, gt)
    return outT.T[None]
```

```python
import os
import numpy as np
import jax
import jax.numpy as jnp
import jax.experimental.pallas as pl
import jax.experimental.pallas.tpu as pltpu

S, D, F, KS = 2048, 448, 1792, 4
BL = 128
NB = S // BL
DP = 512
EPS = 1e-5
TM = 256
NT = S // TM
BPT = TM // BL
FC = 256
NFC = F // FC
SPC = FC // 128
LSTEP = int(os.environ.get('LSTEP', 8))
NP = D // 8
RG = int(os.environ.get('RG', 64))
f32, bf16, u32 = jnp.float32, jnp.bfloat16, jnp.uint32

KV_TIE = int(os.environ.get('KV_TIE', 4))
DFT_BACK = int(os.environ.get('DFT_BACK', 1))
KV0_FIRST = int(os.environ.get('KV0_FIRST', 20))
END_SLACK = float(os.environ.get('END_SLACK', 0.3))
NRQ = int(os.environ.get('NRQ', 4))
RQ = D // NRQ
W1T_LAG = int(os.environ.get('W1T_LAG', 3))
L_DFT = float(os.environ.get('L_DFT', 20.0))

SEM_G = 0
SEM_H = 12
SEM_O = 14
NSEM = 15
AK, AV, AQ = 0, 1, 2


def _pack_np(a):
    u = np.ascontiguousarray(a, dtype=np.float32).view(np.uint32)
    b = (u + 0x7FFF + ((u >> 16) & 1)) >> 16
    return (b[..., 0::2, :] | (b[..., 1::2, :] << 16)).astype(np.uint32)


def _dft_consts():
    t = np.arange(BL, dtype=np.float64)[:, None]
    f = np.arange(BL, dtype=np.float64)[None, :]
    th = 2.0 * np.pi * t * (f + 0.5) / (2 * BL)
    ft = np.stack([np.cos(th), -np.sin(th)], axis=0)
    gt = np.concatenate([np.cos(th).T, -np.sin(th).T], axis=0) / BL
    return jnp.asarray(_pack_np(ft)), jnp.asarray(_pack_np(gt))


def _gelu2(x):
    c = 0.7978845608028654
    return x * (1.0 + jnp.tanh(x * (c + (c * 0.044715) * (x * x))))


def _col(vec_row):
    return jnp.broadcast_to(vec_row, (128, D)).T


def _pk(x):
    return pltpu.bitcast(x, u32)


def _upk(x):
    return pltpu.bitcast(x, bf16)


def _pack2(a, b):
    return pltpu.bitcast(pltpu.pack_elementwise([a, b], packed_dtype=bf16), u32)


def _pack_groups(x):
    n = x.shape[0] // 16
    return jnp.concatenate([_pack2(x[16 * m:16 * m + 8], x[16 * m + 8:16 * m + 16]) for m in range(n)], axis=0)


def _rowsum8(x, tie=None):
    n = x.shape[0] // 8
    acc = x[0:8] if tie is None else tie(x[0:8])
    for i in range(1, n):
        acc = acc + x[i * 8:(i + 1) * 8]
    return acc


def _mean8(acc8):
    return jnp.broadcast_to(jnp.sum(acc8, axis=0, keepdims=True) * (1.0 / D), (8, 128))


def _tile8(stat8, n):
    return jnp.concatenate([stat8] * (n // 8), axis=0)


def _kernel(q_hbm, k_hbm, v_hbm, sk_hbm, ssm_hbm, d_hbm, w1_hbm, b1_hbm, w2_hbm, b2_hbm,
            ft_hbm, gt_hbm, o_hbm,
            q_ref, k_ref, v_ref, sk_ref, ssm_ref, d_ref, w1_ref, b1_ref, w2_ref, b2_ref,
            ft_ref, gt_ref, o_ref,
            cols_ref, w1t_ref, uk_ref, kraw_ref, yh_ref, kv_ref, h_ref, xa_ref, acc_ref,
            st_ref, g_ref, w2p_ref, tmp_ref, vec_ref, sems):
    def col_slice(i, w):
        if isinstance(i, int):
            return pl.ds(i * w, w)
        return pl.ds(pl.multiple_of(i * w, w), w)

    def cp(src, dst, sem):
        return pltpu.make_async_copy(src, dst, sems.at[sem])

    def q_in(t, sem):
        return [cp(q_hbm.at[:, col_slice(t, TM)], q_ref.at[t], sem)]

    def kv_in(t, sem):
        return [cp(k_hbm.at[:, col_slice(t, TM)], k_ref.at[t], sem),
                cp(v_hbm.at[:, col_slice(t, TM)], v_ref.at[t], sem)]

    def ssm_in(t, sem):
        return [cp(ssm_hbm.at[:, col_slice(t, TM)], ssm_ref.at[t], sem)]

    def tile_in(t, sem):
        return kv_in(t, sem) + ssm_in(t, sem)

    def w1_in(c0, c1, sem):
        sl = pl.ds(c0 * FC, (c1 - c0) * FC)
        return [cp(w1_hbm.at[:, sl], w1_ref.at[:, sl], sem)]

    def w2_in(c0, c1, sem):
        sl = pl.ds(c0 * FC, (c1 - c0) * FC)
        return [cp(w2_hbm.at[:, sl], w2_ref.at[:, sl], sem)]

    def out_cp(t, sem):
        return [cp(o_ref.at[t * BPT + a], o_hbm.at[:, col_slice(t * BPT + a, BL)], sem) for a in range(BPT)]

    def out_rows(t, rq):
        rs = pl.ds(rq * RQ, RQ)
        return [cp(o_ref.at[t * BPT + a, rs, :], o_hbm.at[rs, col_slice(t * BPT + a, BL)], SEM_O) for a in range(BPT)]

    G = [
        [cp(s, d, SEM_G) for s, d in [(sk_hbm, sk_ref), (d_hbm, d_ref), (b2_hbm, b2_ref), (b1_hbm, b1_ref)]],
        kv_in(0, SEM_G + 1),
        [cp(ft_hbm, ft_ref, SEM_G + 2)] + ssm_in(0, SEM_G + 2),
        [cp(gt_hbm, gt_ref, SEM_G + 3)] + q_in(0, SEM_G + 3),
        w1_in(0, 3, SEM_G + 4),
        w1_in(3, 7, SEM_G + 5),
        tile_in(1, SEM_G + 6),
        q_in(1, SEM_G + 7) + w2_in(0, 4, SEM_G + 7),
        w2_in(4, 7, SEM_G + 8) + kv_in(2, SEM_G + 8),
        ssm_in(2, SEM_G + 9) + kv_in(3, SEM_G + 9),
        q_in(2, SEM_G + 10) + ssm_in(3, SEM_G + 10) + kv_in(4, SEM_G + 10),
        ssm_in(4, SEM_G + 11) + q_in(3, SEM_G + 11) + tile_in(5, SEM_G + 11),
    ]
    H = [q_in(4, SEM_H) + q_in(5, SEM_H) + tile_in(6, SEM_H) + tile_in(7, SEM_H),
         q_in(6, SEM_H + 1) + q_in(7, SEM_H + 1)]
    for grp in G + H:
        for c in grp:
            c.start()

    def wait(copies):
        for c in copies:
            c.wait()

    def prep_cols():
        def init(i, c):
            z8 = jnp.zeros((8, 128), f32)
            zu = jnp.zeros((8, 128), u32)
            uk_ref[0, i, 0] = z8
            kraw_ref[i, 0:8, :] = z8
            st_ref[i, 0] = z8
            g_ref[i, 0, 0, 0:8, :] = zu
            h_ref[i, 0, 0:8, :] = z8
            xa_ref[i, 0, 0:8, :] = zu
            w2p_ref[i, 0:8, :] = zu
            w1t_ref[i, 0:8, :] = zu
            tmp_ref[i, 0, 0:8, :] = z8
            yh_ref[i, 0, 0:16, :] = jnp.zeros((16, 128), bf16)
            kv_ref[pl.ds(pl.multiple_of(i * 8, 8), 8), :] = zu
            return c
        jax.lax.fori_loop(0, 2, init, 0)
        sk = sk_ref[...].astype(f32)
        rows = [sk[j:j + 1, :] for j in range(KS)] + [d_ref[...].astype(f32).reshape(1, D),
                                                      b2_ref[...].astype(f32).reshape(1, D)]
        for j, r in enumerate(rows):
            vec_ref[j] = jnp.broadcast_to(r, (16, D)).astype(bf16)

        def mk(i, c):
            for j in range(2):
                cols_ref[2 * i + j] = jnp.concatenate([vec_ref[2 * i + j].astype(f32)] * 8, axis=0).T
            return c
        jax.lax.fori_loop(0, 3, mk, 0)

    def prep_more():
        rowt = jax.lax.broadcasted_iota(jnp.int32, (DP - D, 128), 0)
        tail = jnp.where(rowt == 0, 1.0, 0.0).astype(bf16)
        for par in range(2):
            for b in range(BPT):
                xa_ref[par, b, D // 2:DP // 2, :] = _pk(tail)

    def w1t_gen(c0, c1):
        row = jax.lax.broadcasted_iota(jnp.int32, (DP - D, 128), 0)

        def finish(j, kt, tie):
            for m in range(4):
                rows = [tmp_ref[j, kt, pl.ds(32 * m + o, 8, stride=4), :] for o in range(4)]
                if m == 3:
                    rows[3] = tie(rows[3])
                base = j * 64 + m * 16
                w1t_ref[kt, base:base + 8, :] = _pack2(rows[0], rows[2])
                w1t_ref[kt, base + 8:base + 16, :] = _pack2(rows[1], rows[3])
        pend = []
        for j in range(c0 * SPC, c1 * SPC):
            for kt in range(DP // 128):
                tie = yield
                r0, r1 = kt * 128, min((kt + 1) * 128, D)
                w = w1_ref[r0:r1, j * 128:(j + 1) * 128].astype(f32)
                w = jnp.concatenate([w[:-8], tie(w[-8:])], axis=0)
                blk = _upk(_pack_groups(w)).astype(f32)
                if r1 - r0 < 128:
                    b1row = jnp.broadcast_to(b1_ref[j:j + 1, :].astype(f32), (DP - D, 128))
                    blk = jnp.concatenate([blk, jnp.where(row == 0, b1row, 0.0)], axis=0)
                tmp_ref[j, kt] = blk.T
                pend.append((j, kt))
                if len(pend) > W1T_LAG:
                    finish(*pend.pop(0), tie)
        for _ in range(W1T_LAG):
            tie = yield
            if pend:
                finish(*pend.pop(0), tie)

    def w1t_units(c0, c1):
        return (c1 - c0) * SPC * (DP // 128) + W1T_LAG

    def put(slot, sub, val):
        uk_ref[slot, :, sub] = val.reshape(NP, 8, 128)

    def kv_gen(t):
        def halves(w):
            return (pltpu.bitcast(w << 16, f32), pltpu.bitcast(w & jnp.uint32(0xFFFF0000), f32))
        for r0 in range(0, D, 16):
            tie = yield
            r1 = r0 + 16
            kc = [_pk(k_ref[t, r0:r1, a * BL:(a + 1) * BL]) for a in range(BPT)]
            prev = jnp.zeros((8, 128), u32) if t == 0 else _pk(k_ref[t - 1, r0:r1, TM - 128:TM])
            kf = jnp.concatenate([prev] + kc, axis=1)
            if KV_TIE & 1:
                kf = pltpu.bitcast(jnp.concatenate(
                    [tie(pltpu.bitcast(kf[:, i * 128:(i + 1) * 128], f32)) for i in range(BPT + 1)], axis=1), u32)
            sh = [kf[:, 128:]] + [pltpu.roll(kf, j, 1)[:, 128:] for j in range(1, KS)]
            vw = jnp.concatenate([_pk(v_ref[t, r0:r1, a * BL:(a + 1) * BL]) for a in range(BPT)], axis=1)
            res = []
            for o in range(2):
                acc = None
                for j in range(KS):
                    cj = cols_ref[j, pl.ds(r0 + o, 8, stride=2), :]
                    if j == 0 and KV_TIE & 4:
                        cj = tie(cj)
                    cj = jnp.tile(cj, (1, BPT))
                    term = halves(sh[j])[o] * cj
                    acc = term if acc is None else acc + term
                res.append(acc * halves(vw)[o])
            for a in range(BPT):
                cs = slice(a * BL, (a + 1) * BL)
                pk = _pack2(res[0][:, cs], res[1][:, cs])
                if KV_TIE & 2:
                    pk = pltpu.bitcast(tie(pltpu.bitcast(pk, f32)), u32)
                kv_ref[(a * D + r0) // 2:(a * D + r1) // 2, :] = pk

    KV_UNITS = D // 16

    def dft(t):
        lane = jax.lax.broadcasted_iota(jnp.int32, (16, 128), 1)
        sgn = jnp.where((lane & 1) == 0, 1.0, -1.0).astype(f32)
        ft = jnp.concatenate([_upk(ft_ref[0]), _upk(ft_ref[1])], axis=1)
        lk = jnp.concatenate([ssm_ref[t, r0:r0 + 16, a * BL:(a + 1) * BL] for r0 in range(0, D, 16) for a in range(BPT)],
                             axis=0)
        sk_ = jnp.dot(lk, ft, preferred_element_type=f32)
        su = jnp.dot(_upk(kv_ref[...]), ft, preferred_element_type=f32)
        for r0 in range(0, D, 16):
            ps = slice(r0 // 8, r0 // 8 + 2)
            for a in range(BPT):
                blk = t * BPT + a
                o = BPT * r0 + 16 * a
                p = sk_[o:o + 16, :128]
                q = sk_[o:o + 16, 128:]
                if blk == 0:
                    c = p + cols_ref[4, r0:r0 + 16, :]
                    d = q
                else:
                    if a == 0:
                        pp = kraw_ref[0, r0:r0 + 16, :]
                        qq = kraw_ref[1, r0:r0 + 16, :]
                    c = p - qq
                    d = q + pp
                uk_ref[blk, ps, 3] = c.reshape(2, 8, 128)
                uk_ref[blk, ps, 4] = (d - c).reshape(2, 8, 128)
                uk_ref[blk, ps, 5] = (c + d).reshape(2, 8, 128)
                if blk < NB - 1:
                    pp = sgn * p
                    qq = sgn * q
                    if a == BPT - 1:
                        kraw_ref[0, r0:r0 + 16, :] = pp
                        kraw_ref[1, r0:r0 + 16, :] = qq
        for a in range(BPT):
            ur = su[a * D:(a + 1) * D, :128]
            ui = su[a * D:(a + 1) * D, 128:]
            blk = t * BPT + a + 1
            put(blk, 0, ur + ui)
            put(blk, 1, ur)
            put(blk, 2, ui)
        return su

    def mac_gen(t, nlag, tmin=None):
        static = isinstance(t, int)
        a_last = t * BPT + BPT - 1
        if static:
            uslot = [max(a_last - e + 1, 0) for e in range(nlag)]
            kslot = [min(dl, a_last) for dl in range(nlag)]
        else:
            amin = tmin * BPT + BPT - 1
            uslot = [jnp.maximum(a_last - e + 1, 0) if amin - e + 1 < 0 else a_last - e + 1 for e in range(nlag)]
            kslot = [jnp.minimum(dl, a_last) if dl > amin else dl for dl in range(nlag)]
        for p in range(NP):
            if p % 2 == 0:
                re_rows = [[] for _ in range(BPT)]
                im_rows = [[] for _ in range(BPT)]
            res = [None] * BPT
            for comp, sign in ((0, 1), (2, -1), (1, 1)):
                accs = [None] * BPT if comp == 0 else list(res)
                us = {}
                for l0 in range(0, nlag, LSTEP):
                    tie = yield
                    l1 = min(l0 + LSTEP, nlag)
                    for dl in range(l0, l1):
                        kx = uk_ref[kslot[dl], p, 3 + comp]
                        if dl == l0:
                            kx = tie(kx)
                        for i in range(BPT):
                            e = dl + BPT - 1 - i
                            if e >= nlag:
                                continue
                            if e not in us:
                                us[e] = uk_ref[uslot[e], p, comp]
                            pr = us[e] * kx
                            if accs[i] is None:
                                accs[i] = pr
                            elif sign > 0:
                                accs[i] = accs[i] + pr
                            else:
                                accs[i] = accs[i] - pr
                for i in range(BPT):
                    if comp == 0:
                        res[i] = accs[i]
                    elif comp == 2:
                        re_rows[i].append(accs[i])
                    else:
                        im_rows[i].append(accs[i])
            if p % 2 == 1:
                rr = slice((p // 2) * 16, (p // 2) * 16 + 16)
                for i in range(BPT):
                    yh_ref[i, 0, rr, :] = jnp.concatenate(re_rows[i], axis=0).astype(bf16)
                    yh_ref[i, 1, rr, :] = jnp.concatenate(im_rows[i], axis=0).astype(bf16)

    def mac_units(nlag):
        return NP * 3 * (-(-nlag // LSTEP))

    def inv(b):
        yh = jnp.concatenate([yh_ref[b, 0], yh_ref[b, 1]], axis=1)
        return jnp.dot(yh, _upk(gt_ref[...]), preferred_element_type=f32)

    def xstats_gen(t):
        for b in range(BPT):
            cs = slice(b * BL, (b + 1) * BL)
            acc = None
            for r0 in range(0, D, RG):
                tie = yield
                s = _rowsum8(q_ref[t, r0:r0 + RG, cs].astype(f32), tie)
                acc = s if acc is None else acc + s
            st_ref[b, 0] = _mean8(acc)
        for b in range(BPT):
            cs = slice(b * BL, (b + 1) * BL)
            acc = None
            for r0 in range(0, D, RG):
                tie = yield
                xc = q_ref[t, r0:r0 + RG, cs].astype(f32) - _tile8(tie(st_ref[b, 0]), RG)
                s = _rowsum8(xc * xc)
                acc = s if acc is None else acc + s
            st_ref[b, 1] = jax.lax.rsqrt(_mean8(acc) + EPS)

    XSTAT_UNITS = 2 * BPT * (D // RG)

    def pass_c(t, par, b, y):
        cs = slice(b * BL, (b + 1) * BL)
        x = q_ref[t, :, cs].astype(f32)
        xc = x - _tile8(st_ref[b, 0], D)
        h = x + xc * (y * _tile8(st_ref[b, 1], D))
        h_ref[par, b] = h
        return _mean8(_rowsum8(h))

    def hln_gen(par, m1):
        r1 = [None] * BPT
        m2 = [None] * BPT
        r2 = [None] * BPT
        for b in range(BPT):
            acc = None
            for r0 in range(0, D, RG):
                tie = yield
                hc = h_ref[par, b, r0:r0 + RG, :] - _tile8(tie(m1[b]), RG)
                s = _rowsum8(hc * hc)
                acc = s if acc is None else acc + s
            r1[b] = jax.lax.rsqrt(_mean8(acc) + EPS)
        for b in range(BPT):
            acc = None
            for r0 in range(0, D, RG):
                tie = yield
                zz = (h_ref[par, b, r0:r0 + RG, :] - _tile8(tie(m1[b]), RG)) * _tile8(r1[b], RG)
                s = _rowsum8(zz)
                acc = s if acc is None else acc + s
            m2[b] = _mean8(acc)
        for b in range(BPT):
            acc = None
            for r0 in range(0, D, RG):
                tie = yield
                zc = (h_ref[par, b, r0:r0 + RG, :] - _tile8(tie(m1[b]), RG)) * _tile8(r1[b], RG) - _tile8(m2[b], RG)
                s = _rowsum8(zc * zc)
                acc = s if acc is None else acc + s
            r2[b] = jax.lax.rsqrt(_mean8(acc) + EPS)
        for b in range(BPT):
            for r0 in range(0, D, RG):
                tie = yield
                zc = (h_ref[par, b, r0:r0 + RG, :] - _tile8(tie(m1[b]), RG)) * _tile8(r1[b], RG) - _tile8(m2[b], RG)
                xa_ref[par, b, r0 // 2:(r0 + RG) // 2, :] = _pack_groups(zc * _tile8(r2[b], RG))

    HLN_UNITS = 4 * BPT * (D // RG)

    def run_all(gen):
        next(gen)
        while True:
            try:
                gen.send(lambda x: x)
            except StopIteration:
                return

    NCAND = {'mm1': 64, 'mm2': 56, 'inv': 56, 'dft': 112}
    LOAD = {'mm1': 10.0, 'mm2': 4.5, 'inv': 18.0, 'dft': L_DFT}

    def s_mac(t, p0, p1):
        nlag = BPT * (t + 1)
        n = mac_units(nlag)
        return (lambda: mac_gen(t, nlag), n, (NP * 6.0 * (2 * nlag - 1) + 340) / n + 1, p0, p1)

    def s_hln(par, p0, p1):
        return (lambda: hln_gen(par, state['m1']), HLN_UNITS, 34.0, p0, p1)

    def s_xs(t, p0, p1):
        return (lambda: xstats_gen(t), XSTAT_UNITS, 26.0, p0, p1)

    def s_kv(t, p0, p1):
        return (lambda: kv_gen(t), KV_UNITS, 70.0, p0, p1)

    def s_w1t(c0, c1, p0, p1):
        return (lambda: w1t_gen(c0, c1), w1t_units(c0, c1), 60.0, p0, p1)

    state = {}

    def segment(phases, streams):
        always = gt_ref[0:8, :] != jnp.uint32(0x7FC17FC1)
        pos, load, keys = [], [], []
        for pi, ph in enumerate(phases):
            n = NCAND.get(ph[0], 0)
            for c in range(n):
                pos.append(pi + (c + 0.5) / n)
                load.append(LOAD[ph[0]])
                keys.append((pi, c))
        pos, load = np.array(pos), np.array(load, dtype=np.float64)
        plan = {}
        for si, (mk, n, cost, p0, p1) in enumerate(streams):
            idx = np.nonzero((pos >= p0) & (pos <= p1))[0]
            lo, hi = 0.0, 1000.0
            for _ in range(60):
                mid = 0.5 * (lo + hi)
                if np.maximum(mid - load[idx], 0).sum() < n * cost:
                    lo = mid
                else:
                    hi = mid
            add = np.maximum(hi - load[idx], 0) + 1e-9
            load[idx] += add
            if os.environ.get('SHOW_LOAD'):
                print('stream', si, 'units', n, 'level', round(hi / 8, 2))
            cums = np.cumsum(add) / add.sum()
            holder = {}

            def fire(val, mk=mk, holder=holder):
                if 'g' not in holder:
                    holder['g'] = mk()
                    next(holder['g'])
                try:
                    holder['g'].send(lambda x: jnp.where(always, x, val))
                except StopIteration:
                    pass
            for u in range(n):
                ci = idx[min(int(np.searchsorted(cums, (u + 0.5) / n)), len(idx) - 1)]
                plan.setdefault(keys[ci], []).append(fire)

        def fire_all(pi, getter):
            for c in range(NCAND[phases[pi][0]]):
                for fire in plan.get((pi, c), []):
                    fire(getter(c))

        for pi, ph in enumerate(phases):
            kind = ph[0]
            if kind == 'mm1':
                _, par, j = ph
                xa = jnp.concatenate([_upk(xa_ref[par, b]) for b in range(BPT)], axis=1)
                w1c = jnp.concatenate([_upk(w1t_ref[kt, j * FC // 2:(j + 1) * FC // 2, :])
                                       for kt in range(DP // 128)], axis=1)
                pre = jnp.dot(w1c, xa, preferred_element_type=f32)
                g = _gelu2(pre)
                for b in range(BPT):
                    gb = g[:, b * BL:(b + 1) * BL]
                    for m in range(FC // 32):
                        r = 32 * m
                        g_ref[par, j, b, 16 * m:16 * m + 8, :] = _pack2(gb[r:r + 8], gb[r + 16:r + 24])
                        g_ref[par, j, b, 16 * m + 8:16 * m + 16, :] = _pack2(gb[r + 8:r + 16], gb[r + 24:r + 32])
                fire_all(pi, lambda c: pre[(c % 32) * 8:(c % 32) * 8 + 8, (c // 32) * 128:(c // 32) * 128 + 128])
            elif kind == 'mm2':
                _, par, j, raw = ph
                if raw:
                    slabs = [w2_ref[:, (j * SPC + kt) * 128:(j * SPC + kt + 1) * 128] for kt in range(SPC)]
                    for kt in range(SPC):
                        w2p_ref[j * SPC + kt] = _pk(slabs[kt])
                else:
                    slabs = [_upk(w2p_ref[j * SPC + kt]) for kt in range(SPC)]
                gj = jnp.concatenate([_upk(g_ref[par, j, b]) for b in range(BPT)], axis=1)
                part = jnp.dot(jnp.concatenate(slabs, axis=1), gj, preferred_element_type=f32)
                state['acc'] = part if j == 0 else state['acc'] + part
                fire_all(pi, lambda c: part[c * 8:c * 8 + 8, 0:128])
            elif kind == 'inv':
                _, t, par = ph
                ys = [inv(b) for b in range(BPT)]
                state['m1'] = [pass_c(t, par, b, ys[b]) for b in range(BPT)]
                fire_all(pi, lambda c: ys[0][c * 8:c * 8 + 8, :])
            elif kind == 'dft':
                _, t = ph
                su = dft(t)
                fire_all(pi, lambda c: su[c * 8:c * 8 + 8, 0:128])
            elif kind == 'out':
                _, t, par = ph
                acc = state['acc']
                for b in range(BPT):
                    o_ref[t * BPT + b] = (0.5 * acc[:, b * BL:(b + 1) * BL]
                                          + (h_ref[par, b] + cols_ref[5])).astype(o_ref.dtype)
            elif kind == 'out_send':
                _, t, par = ph
                acc = state['acc']
                for rq in range(NRQ):
                    rs = slice(rq * RQ, (rq + 1) * RQ)
                    for b in range(BPT):
                        o_ref[t * BPT + b, rs, :] = (0.5 * acc[rs, b * BL:(b + 1) * BL]
                                                     + (h_ref[par, b, rs, :] + cols_ref[5, rs, :])).astype(o_ref.dtype)
                    for c in out_rows(t, rq):
                        c.start()
            elif kind == 'acc_store':
                acc_ref[ph[1]] = state['acc']
            elif kind == 'acc_load':
                state['acc'] = acc_ref[ph[1]]
            elif kind == 'send':
                _, t, sem = ph
                for c in out_cp(t, sem):
                    c.start()

    def mlp_phases(par, j0, j1):
        ph = []
        for j in range(j0, j1):
            if j < NFC:
                ph.append(('mm1', par, j))
            if j > 0:
                ph.append(('mm2', par, j - 1, False))
        return ph

    def steady(tiles, dfts, last_partial=None):
        phases, streams = [], []
        dfts = list(dfts)
        for t in tiles:
            par = t % 2
            p0 = len(phases)
            phases += [('inv', t + 1, 1 - par)] + mlp_phases(par, 0, NFC + 1)
            if dfts:
                td = dfts.pop(0)
                pd = len(phases) - DFT_BACK
                phases.insert(pd, ('dft', td))
                streams.append(s_kv(td, p0 + 1.0, pd - 0.5))
            end = len(phases) - 0.4
            streams.append(s_hln(1 - par, p0 + 1.3, end - END_SLACK))
            streams.append(s_xs(t + 2, p0 + 1.3, end - END_SLACK))
            streams.append(s_mac(t + 2, p0 + 1.0, end - END_SLACK))
            phases += [('out', t, par), ('send', t, SEM_O)]
        if last_partial is not None:
            p0 = len(phases)
            phases += [('inv', 7, 1)] + mlp_phases(0, 0, NFC + 1) + [('out', 6, 0), ('send', 6, SEM_O)]
            streams.append(s_hln(1, p0 + 1.3, p0 + float(os.environ.get('H7', 4.0))))
            phases += mlp_phases(1, 0, NFC + 1) + [('out_send', 7, 1)]
        segment(phases, streams)

    wait(G[0])
    prep_cols()
    prep_more()
    wait(G[1])
    kv0 = kv_gen(0)
    next(kv0)
    for _ in range(KV0_FIRST):
        kv0.send(lambda x: x)
    wait(G[2])
    for _ in range(KV_UNITS - KV0_FIRST):
        try:
            kv0.send(lambda x: x)
        except StopIteration:
            pass
    dft(0)
    run_all(mac_gen(0, BPT))
    wait(G[3])
    run_all(xstats_gen(0))
    m1_0 = [pass_c(0, 0, b, inv(b)) for b in range(BPT)]
    wait(G[4])
    run_all(hln_gen(0, m1_0))
    run_all(w1t_gen(0, 2))
    segment([('mm1', 0, 0), ('mm1', 0, 1)], [s_w1t(2, 3, 0.2, 1.4)])
    wait(G[5])
    segment([('mm1', 0, 2), ('mm1', 0, 3), ('mm1', 0, 4)],
            [s_w1t(3, 5, 0.0, 1.2), s_w1t(5, 7, 1.0, 2.4)])
    wait(G[6])
    segment([('mm1', 0, 5), ('mm1', 0, 6), ('dft', 1)], [s_kv(1, 0.0, 1.8)])
    wait(G[7])
    segment([('mm2', 0, j, True) for j in range(4)], [s_xs(1, 0.0, float(os.environ.get('S6E', 2.6))), s_mac(1, 0.0, float(os.environ.get('S6E', 2.6)))])
    wait(G[8])
    segment([('inv', 1, 1)] + [('mm2', 0, j, True) for j in range(4, 7)] + [('out', 0, 0), ('send', 0, SEM_O)],
            [s_hln(1, 1.2, 3.7), s_kv(2, 0.3, 3.7)])
    wait(G[9])
    segment([('dft', 2), ('mm1', 1, 0), ('mm1', 1, 1)], [s_kv(3, float(os.environ.get('KV3', 1.0)), 2.7)])
    wait(G[10])
    segment([('dft', 3), ('mm2', 1, 0, False)] + mlp_phases(1, 2, 4), [s_kv(4, 2.2, 5.6), s_xs(2, 0.0, 5.4), s_mac(2, 0.0, 5.6)])
    wait(G[11])
    segment([('inv', 2, 0), ('dft', 4)] + mlp_phases(1, 4, 7) + [('dft', 5), ('mm2', 1, 6, False), ('out', 1, 1), ('send', 1, SEM_O)],
            [s_kv(5, 3.2, 7.5), s_hln(0, 1.3, 9.6), s_xs(3, 1.3, 9.6), s_mac(3, 1.0, 9.6)])
    wait(H[0])
    steady([2, 3], [6, 7])
    wait(H[1])
    JS = 3
    steady([4, 5], [], (6, JS))

    for t in range(NT - 1):
        wait(out_cp(t, SEM_O))
    for t in range(NT - 1, NT):
        for rq in range(NRQ):
            wait(out_rows(t, rq))


@jax.jit
def pallas_sequential_preLN__ssm_conv_h3__mixer_channel_mlp__prompt_kernel(
    A_q, A_k, A_v, A_shift_k, A_ssm_k, A_ssm_D, B_x, B_w1, B_b1, B_w2, B_b2,
):
    ft, gt = _dft_consts()
    any_spec = pl.BlockSpec(memory_space=pl.ANY)
    outT = pl.pallas_call(
        _kernel,
        out_shape=jax.ShapeDtypeStruct((D, S), bf16),
        in_specs=[any_spec] * 12,
        out_specs=any_spec,
        scratch_shapes=[
            pltpu.VMEM((NT, D, TM), bf16),
            pltpu.VMEM((NT, D, TM), bf16),
            pltpu.VMEM((NT, D, TM), bf16),
            pltpu.VMEM((KS, D), bf16),
            pltpu.VMEM((NT, D, TM), bf16),
            pltpu.VMEM((D,), bf16),
            pltpu.VMEM((D, F), bf16),
            pltpu.VMEM((F // 128, 128), bf16),
            pltpu.VMEM((D, F), bf16),
            pltpu.VMEM((D,), bf16),
            pltpu.VMEM((2, BL // 2, BL), u32),
            pltpu.VMEM((BL, BL), u32),
            pltpu.VMEM((NB, D, BL), bf16),
            pltpu.VMEM((6, D, 128), f32),
            pltpu.VMEM((DP // 128, F // 2, 128), u32),
            pltpu.VMEM((NB + 1, NP, 6, 8, 128), f32),
            pltpu.VMEM((2, D, 128), f32),
            pltpu.VMEM((BPT, 2, D, 128), bf16),
            pltpu.VMEM((BPT * D // 2, 128), u32),
            pltpu.VMEM((2, BPT, D, BL), f32),
            pltpu.VMEM((2, BPT, DP // 2, BL), u32),
            pltpu.VMEM((2, D, TM), f32),
            pltpu.VMEM((BPT, 2, 8, 128), f32),
            pltpu.VMEM((2, NFC, BPT, FC // 2, BL), u32),
            pltpu.VMEM((F // 128, D // 2, 128), u32),
            pltpu.VMEM((F // 128, DP // 128, 128, 128), f32),
            pltpu.VMEM((6, 16, D), bf16),
            pltpu.SemaphoreType.DMA((NSEM,)),
        ],
        compiler_params=pltpu.CompilerParams(vmem_limit_bytes=110 * 1024 * 1024),
    )(A_q[0].T, A_k[0].T, A_v[0].T, A_shift_k.T, A_ssm_k, A_ssm_D, B_w1,
      B_b1.reshape(F // 128, 128), B_w2.T, B_b2, ft, gt)
    return outT.T[None]
```

```python
import numpy as np
import jax
import jax.numpy as jnp
import jax.experimental.pallas as pl
import jax.experimental.pallas.tpu as pltpu

S, D, F, KS = 2048, 448, 1792, 4
BL = 128
NB = S // BL
DP = 512
EPS = 1e-5
TM = 256
NT = S // TM
BPT = TM // BL
FC = 256
NFC = F // FC
SPC = FC // 128
NP = D // 8
LSTEP = 8
RG = 64
NKV = 3
NRQ = 4
RQ = D // NRQ
W1T_LAG = 3
KV0_FIRST = 20
JS = 5
DFT_POS = (10, 12, 14)
f32, bf16, u32 = jnp.float32, jnp.bfloat16, jnp.uint32

NGRP = 13
SEM_O = NGRP
NSEM = NGRP + 1


def _pack_np(a):
    u = np.ascontiguousarray(a, dtype=np.float32).view(np.uint32)
    b = (u + 0x7FFF + ((u >> 16) & 1)) >> 16
    return (b[..., 0::2, :] | (b[..., 1::2, :] << 16)).astype(np.uint32)


def _dft_consts():
    t = np.arange(BL, dtype=np.float64)[:, None]
    f = np.arange(BL, dtype=np.float64)[None, :]
    th = 2.0 * np.pi * t * (f + 0.5) / (2 * BL)
    ft = np.stack([np.cos(th), -np.sin(th)], axis=0)
    gt = np.concatenate([np.cos(th).T, -np.sin(th).T], axis=0) / BL
    return jnp.asarray(_pack_np(ft)), jnp.asarray(_pack_np(gt))


def _gelu2(x):
    c = 0.7978845608028654
    return x * (1.0 + jnp.tanh(x * (c + (c * 0.044715) * (x * x))))


def _col(vec_row):
    return jnp.broadcast_to(vec_row, (128, D)).T


def _pk(x):
    return pltpu.bitcast(x, u32)


def _upk(x):
    return pltpu.bitcast(x, bf16)


def _rowsum8(x, tie=None):
    acc = x[0:8] if tie is None else tie(x[0:8])
    for i in range(1, x.shape[0] // 8):
        acc = acc + x[i * 8:(i + 1) * 8]
    return acc


def _mean8(acc8):
    return jnp.broadcast_to(jnp.sum(acc8, axis=0, keepdims=True) * (1.0 / D), (8, 128))


def _tile8(stat8, n):
    return jnp.concatenate([stat8] * (n // 8), axis=0)


def _kernel(q_hbm, k_hbm, v_hbm, sk_hbm, ssm_hbm, d_hbm, w1_hbm, b1_hbm, w2_hbm, b2_hbm,
            ft_hbm, gt_hbm, o_hbm,
            q_ref, k_ref, v_ref, sk_ref, ssm_ref, d_ref, w1_ref, b1_ref, w2_ref, b2_ref,
            ft_ref, gt_ref, o_ref,
            cols_ref, w1t_ref, uk_ref, kraw_ref, yh_ref, kv_ref, h_ref, xa_ref, acc_ref,
            st_ref, w2p_ref, g_ref, sems):
    g_w, xa_w, w1t_w, yh_w, kv_w = (r.bitcast(u32) for r in (g_ref, xa_ref, w1t_ref, yh_ref, kv_ref))
    done = set()
    state = {}

    def col_slice(i, w):
        if isinstance(i, int):
            return pl.ds(i * w, w)
        return pl.ds(pl.multiple_of(i * w, w), w)

    def q_in(t):
        return [(q_hbm.at[:, col_slice(t, TM)], q_ref.at[t])]

    def kv_in(t):
        return [(k_hbm.at[:, col_slice(t, TM)], k_ref.at[t]), (v_hbm.at[:, col_slice(t, TM)], v_ref.at[t])]

    def ssm_in(t):
        return [(ssm_hbm.at[:, col_slice(t, TM)], ssm_ref.at[t])]

    def tile_in(t):
        return kv_in(t) + ssm_in(t)

    def w_in(src, dst, c0, c1):
        sl = pl.ds(c0 * FC, (c1 - c0) * FC)
        return [(src.at[:, sl], dst.at[:, sl])]

    def out_cp(t):
        return [pltpu.make_async_copy(o_ref.at[t * BPT + a], o_hbm.at[:, col_slice(t * BPT + a, BL)],
                                      sems.at[SEM_O]) for a in range(BPT)]

    def out_rows(t, rq):
        rs = pl.ds(rq * RQ, RQ)
        return [pltpu.make_async_copy(o_ref.at[t * BPT + a, rs, :], o_hbm.at[rs, col_slice(t * BPT + a, BL)],
                                      sems.at[SEM_O]) for a in range(BPT)]

    groups = [
        [(sk_hbm, sk_ref), (d_hbm, d_ref), (b2_hbm, b2_ref), (b1_hbm, b1_ref)],
        kv_in(0),
        [(ft_hbm, ft_ref)] + ssm_in(0),
        [(gt_hbm, gt_ref)] + q_in(0),
        w_in(w1_hbm, w1_ref, 0, 3),
        w_in(w1_hbm, w1_ref, 3, 7),
        tile_in(1),
        q_in(1) + w_in(w2_hbm, w2_ref, 0, 4),
        w_in(w2_hbm, w2_ref, 4, 7),
        tile_in(2) + tile_in(3),
        q_in(2) + tile_in(4) + q_in(3),
        q_in(4) + tile_in(5) + tile_in(6) + tile_in(7),
        q_in(5) + q_in(6) + q_in(7),
    ]
    assert len(groups) == NGRP
    G = [[pltpu.make_async_copy(s, d, sems.at[i]) for s, d in grp] for i, grp in enumerate(groups)]
    for grp in G:
        for c in grp:
            c.start()

    def wait(copies):
        for c in copies:
            c.wait()

    def prep():
        def touch(i, c):
            z8 = jnp.zeros((8, 128), f32)
            zb = jnp.zeros((16, 128), bf16)
            uk_ref[0, i, 0] = z8
            kraw_ref[i, 0:8, :] = z8
            st_ref[i, 0] = z8
            g_ref[i, 0, 0, 0:16, :] = zb
            h_ref[i, 0, 0:8, :] = z8
            xa_ref[i, 0, 0:16, :] = zb
            w2p_ref[i, 0:8, :] = jnp.zeros((8, 128), u32)
            w1t_ref[i, 0:16, :] = zb
            yh_ref[i, 0, 0:16, :] = zb
            kv_ref[i, 0:16, :] = zb
            return c
        jax.lax.fori_loop(0, 2, touch, 0)
        sk = sk_ref[...].astype(f32)
        for j in range(KS):
            cols_ref[j] = _col(sk[j:j + 1, :])
        cols_ref[4] = _col(d_ref[...].astype(f32).reshape(1, D))
        cols_ref[5] = _col(b2_ref[...].astype(f32).reshape(1, D))
        rowt = jax.lax.broadcasted_iota(jnp.int32, (DP - D, 128), 0)
        tail = jnp.where(rowt == 0, 1.0, 0.0).astype(bf16)
        for par in range(2):
            for b in range(BPT):
                xa_ref[par, b, D:DP, :] = tail

    def w1t_gen(c0, c1):
        row = jax.lax.broadcasted_iota(jnp.int32, (DP - D, 128), 0)

        def finish(j, kt, bt, tie):
            bt = jnp.concatenate([bt[:-8], tie(bt[-8:])], axis=0)
            w1t_ref[kt, j * 128:(j + 1) * 128, :] = bt.astype(bf16)
            done.add(('w1t', j, kt))
        pend = []
        for j in range(c0 * SPC, c1 * SPC):
            for kt in range(DP // 128):
                tie = yield
                r0, r1 = kt * 128, min((kt + 1) * 128, D)
                w = w1_ref[r0:r1, j * 128:(j + 1) * 128].astype(f32)
                blk = jnp.concatenate([w[:-8], tie(w[-8:])], axis=0)
                if r1 - r0 < 128:
                    b1row = jnp.broadcast_to(b1_ref[j:j + 1, :].astype(f32), (DP - D, 128))
                    blk = jnp.concatenate([blk, jnp.where(row == 0, b1row, 0.0)], axis=0)
                pend.append((j, kt, blk.T))
                if len(pend) > W1T_LAG:
                    finish(*pend.pop(0), tie)
        for _ in range(W1T_LAG):
            tie = yield
            if pend:
                finish(*pend.pop(0), tie)

    def kv_gen(t):
        assert t < NKV or ('dft', t - NKV) in done
        for r0 in range(0, D, 16):
            tie = yield
            r1 = r0 + 16
            kc = [_pk(k_ref[t, r0:r1, a * BL:(a + 1) * BL]) for a in range(BPT)]
            prev = jnp.zeros((8, 128), u32) if t == 0 else _pk(k_ref[t - 1, r0:r1, TM - 128:TM])
            kf = jnp.concatenate([prev] + kc, axis=1)
            sh = [kf[:, 128:]] + [pltpu.roll(kf, j, 1)[:, 128:] for j in range(1, KS)]
            acc = None
            for j in range(KS):
                cj = cols_ref[j, r0:r1, :]
                if j == 0:
                    cj = jnp.concatenate([tie(cj[0:8]), tie(cj[8:16])], axis=0)
                term = _upk(sh[j]).astype(f32) * jnp.tile(cj, (1, BPT))
                acc = term if acc is None else acc + term
            kv = acc * v_ref[t, r0:r1, :].astype(f32)
            for a in range(BPT):
                kv_ref[t % NKV, a * D + r0:a * D + r1, :] = kv[:, a * BL:(a + 1) * BL].astype(bf16)
        done.add(('kv', t))

    def dft(t):
        assert ('kv', t) in done and (t == 0 or ('dft', t - 1) in done)
        lane = jax.lax.broadcasted_iota(jnp.int32, (16, 128), 1)
        sgn = jnp.where((lane & 1) == 0, 1.0, -1.0).astype(f32)
        ft = jnp.concatenate([_upk(ft_ref[0]), _upk(ft_ref[1])], axis=1)
        lk = jnp.concatenate([ssm_ref[t, r0:r0 + 16, a * BL:(a + 1) * BL]
                              for r0 in range(0, D, 16) for a in range(BPT)], axis=0)
        sk_ = jnp.dot(lk, ft, preferred_element_type=f32)
        su = jnp.dot(_upk(kv_w[t % NKV]), ft, preferred_element_type=f32)
        for r0 in range(0, D, 16):
            ps = slice(r0 // 8, r0 // 8 + 2)
            for a in range(BPT):
                blk = t * BPT + a
                o = BPT * r0 + 16 * a
                p = sk_[o:o + 16, :128]
                q = sk_[o:o + 16, 128:]
                if blk == 0:
                    c = p + cols_ref[4, r0:r0 + 16, :]
                    d = q
                else:
                    if a == 0:
                        pp = kraw_ref[0, r0:r0 + 16, :]
                        qq = kraw_ref[1, r0:r0 + 16, :]
                    c = p - qq
                    d = q + pp
                uk_ref[blk, ps, 3] = c.reshape(2, 8, 128)
                uk_ref[blk, ps, 4] = (d - c).reshape(2, 8, 128)
                uk_ref[blk, ps, 5] = (c + d).reshape(2, 8, 128)
                if blk < NB - 1:
                    pp = sgn * p
                    qq = sgn * q
                    if a == BPT - 1:
                        kraw_ref[0, r0:r0 + 16, :] = pp
                        kraw_ref[1, r0:r0 + 16, :] = qq
        for a in range(BPT):
            ur = su[a * D:(a + 1) * D, :128]
            ui = su[a * D:(a + 1) * D, 128:]
            slot = t * BPT + a + 1
            uk_ref[slot, :, 0] = (ur + ui).reshape(NP, 8, 128)
            uk_ref[slot, :, 1] = ur.reshape(NP, 8, 128)
            uk_ref[slot, :, 2] = ui.reshape(NP, 8, 128)
        done.add(('dft', t))
        return su

    def mac_gen(t):
        assert ('dft', t) in done and (t == 0 or ('inv', t - 1) in done)
        nlag = BPT * (t + 1)
        for p in range(NP):
            if p % 2 == 0:
                re_rows = [[] for _ in range(BPT)]
                im_rows = [[] for _ in range(BPT)]
            res = [None] * BPT
            for comp, sign in ((0, 1), (2, -1), (1, 1)):
                accs = [None] * BPT if comp == 0 else list(res)
                us = {}
                for l0 in range(0, nlag, LSTEP):
                    tie = yield
                    for dl in range(l0, min(l0 + LSTEP, nlag)):
                        kx = uk_ref[dl, p, 3 + comp]
                        if dl == l0:
                            kx = tie(kx)
                        for i in range(BPT):
                            e = dl + BPT - 1 - i
                            if e >= nlag:
                                continue
                            if e not in us:
                                us[e] = uk_ref[nlag - e, p, comp]
                            pr = us[e] * kx
                            if accs[i] is None:
                                accs[i] = pr
                            elif sign > 0:
                                accs[i] = accs[i] + pr
                            else:
                                accs[i] = accs[i] - pr
                for i in range(BPT):
                    if comp == 0:
                        res[i] = accs[i]
                    elif comp == 2:
                        re_rows[i].append(accs[i])
                    else:
                        im_rows[i].append(accs[i])
            if p % 2 == 1:
                rr = slice((p // 2) * 16, (p // 2) * 16 + 16)
                for i in range(BPT):
                    yh_ref[i, 0, rr, :] = jnp.concatenate(re_rows[i], axis=0).astype(bf16)
                    yh_ref[i, 1, rr, :] = jnp.concatenate(im_rows[i], axis=0).astype(bf16)
        done.add(('mac', t))

    def xstats_gen(t):
        assert t == 0 or ('inv', t - 1) in done
        for b in range(BPT):
            cs = slice(b * BL, (b + 1) * BL)
            acc = None
            for r0 in range(0, D, RG):
                tie = yield
                s = _rowsum8(q_ref[t, r0:r0 + RG, cs].astype(f32), tie)
                acc = s if acc is None else acc + s
            st_ref[b, 0] = _mean8(acc)
        for b in range(BPT):
            cs = slice(b * BL, (b + 1) * BL)
            acc = None
            for r0 in range(0, D, RG):
                tie = yield
                xc = q_ref[t, r0:r0 + RG, cs].astype(f32) - _tile8(tie(st_ref[b, 0]), RG)
                s = _rowsum8(xc * xc)
                acc = s if acc is None else acc + s
            st_ref[b, 1] = jax.lax.rsqrt(_mean8(acc) + EPS)
        done.add(('xs', t))

    def inv_h(t):
        assert ('mac', t) in done and ('xs', t) in done and (t < 2 or ('out', t - 2) in done)
        ys, m1 = [], []
        for b in range(BPT):
            yh = jnp.concatenate([_upk(yh_w[b, 0]), _upk(yh_w[b, 1])], axis=1)
            ys.append(jnp.dot(yh, _upk(gt_ref[...]), preferred_element_type=f32))
        for b in range(BPT):
            x = q_ref[t, :, b * BL:(b + 1) * BL].astype(f32)
            xc = x - _tile8(st_ref[b, 0], D)
            h = x + xc * (ys[b] * _tile8(st_ref[b, 1], D))
            h_ref[t % 2, b] = h
            m1.append(_mean8(_rowsum8(h)))
        state['m1', t] = m1
        done.add(('inv', t))
        return ys[0]

    def hln_gen(t):
        par = t % 2
        m1 = state.pop(('m1', t))
        r1 = [None] * BPT
        m2 = [None] * BPT
        r2 = [None] * BPT

        def hc(b, r0, tie):
            return h_ref[par, b, r0:r0 + RG, :] - _tile8(tie(m1[b]), RG)
        for b in range(BPT):
            acc = None
            for r0 in range(0, D, RG):
                tie = yield
                c = hc(b, r0, tie)
                s = _rowsum8(c * c)
                acc = s if acc is None else acc + s
            r1[b] = jax.lax.rsqrt(_mean8(acc) + EPS)
        for b in range(BPT):
            acc = None
            for r0 in range(0, D, RG):
                tie = yield
                s = _rowsum8(hc(b, r0, tie) * _tile8(r1[b], RG))
                acc = s if acc is None else acc + s
            m2[b] = _mean8(acc)
        for b in range(BPT):
            acc = None
            for r0 in range(0, D, RG):
                tie = yield
                zc = hc(b, r0, tie) * _tile8(r1[b], RG) - _tile8(m2[b], RG)
                s = _rowsum8(zc * zc)
                acc = s if acc is None else acc + s
            r2[b] = jax.lax.rsqrt(_mean8(acc) + EPS)
        for b in range(BPT):
            for r0 in range(0, D, RG):
                tie = yield
                zc = hc(b, r0, tie) * _tile8(r1[b], RG) - _tile8(m2[b], RG)
                xa_ref[par, b, r0:r0 + RG, :] = (zc * _tile8(r2[b], RG)).astype(bf16)
        done.add(('hln', t))

    def step(gen, tie=lambda x: x):
        try:
            gen.send(tie)
            return True
        except StopIteration:
            return False

    def run_all(gen):
        next(gen)
        while step(gen):
            pass

    KV_UNITS = D // 16

    def s_mac(t, p0, p1):
        nlag = BPT * (t + 1)
        n = NP * 3 * (-(-nlag // LSTEP))
        return (lambda: mac_gen(t), n, (NP * 6.0 * (2 * nlag - 1) + 340) / n + 1, p0, p1)

    def s_hln(t, p0, p1):
        return (lambda: hln_gen(t), 4 * BPT * (D // RG), 34.0, p0, p1)

    def s_xs(t, p0, p1):
        return (lambda: xstats_gen(t), 2 * BPT * (D // RG), 26.0, p0, p1)

    def s_kv(t, p0, p1):
        return (lambda: kv_gen(t), KV_UNITS, 70.0, p0, p1)

    def s_w1t(c0, c1, p0, p1):
        return (lambda: w1t_gen(c0, c1), (c1 - c0) * SPC * (DP // 128) + W1T_LAG, 60.0, p0, p1)

    NCAND = {'mm1': 64, 'mm2': 56, 'inv': 56, 'dft': 112}
    LOAD = {'mm1': 10.0, 'mm2': 4.5, 'inv': 18.0, 'dft': 16.0}

    def emit_out(t, rs):
        par = t % 2
        for b in range(BPT):
            o_ref[t * BPT + b, rs, :] = (0.5 * state['acc'][rs, b * BL:(b + 1) * BL]
                                         + (h_ref[par, b, rs, :] + cols_ref[5, rs, :])).astype(o_ref.dtype)

    def segment(phases, streams):
        always = gt_ref[0:8, :] != jnp.uint32(0x7FC17FC1)
        pos, load, keys = [], [], []
        for pi, ph in enumerate(phases):
            n = NCAND.get(ph[0], 0)
            for c in range(n):
                pos.append(pi + (c + 0.5) / n)
                load.append(LOAD[ph[0]])
                keys.append((pi, c))
        pos, load = np.array(pos), np.array(load, dtype=np.float64)
        plan = {}
        for mk, n, cost, p0, p1 in streams:
            idx = np.nonzero((pos >= p0) & (pos <= p1))[0]
            lo, hi = 0.0, 1000.0
            for _ in range(60):
                mid = 0.5 * (lo + hi)
                if np.maximum(mid - load[idx], 0).sum() < n * cost:
                    lo = mid
                else:
                    hi = mid
            add = np.maximum(hi - load[idx], 0) + 1e-9
            load[idx] += add
            cums = np.cumsum(add) / add.sum()
            holder = []

            def fire(val, mk=mk, holder=holder):
                if not holder:
                    holder.append(mk())
                    next(holder[0])
                step(holder[0], lambda x: jnp.where(always, x, val))
            for u in range(n):
                ci = idx[min(int(np.searchsorted(cums, (u + 0.5) / n)), len(idx) - 1)]
                plan.setdefault(keys[ci], []).append(fire)

        def fire_all(pi, getter):
            for c in range(NCAND[phases[pi][0]]):
                for fire in plan.get((pi, c), []):
                    fire(getter(c))

        for pi, ph in enumerate(phases):
            kind, t = ph[0], ph[1]
            static = isinstance(t, int)
            par = t % 2
            if kind == 'mm1':
                j = ph[2]
                assert not static or ('hln', t) in done
                assert all(('w1t', jj, kt) in done for jj in range(j * SPC, (j + 1) * SPC) for kt in range(4))
                xa = jnp.concatenate([_upk(xa_w[par, b]) for b in range(BPT)], axis=1)
                w1c = jnp.concatenate([_upk(w1t_w[kt, j * FC // 2:(j + 1) * FC // 2, :])
                                       for kt in range(DP // 128)], axis=1)
                pre = jnp.dot(w1c, xa, preferred_element_type=f32)
                g = _gelu2(pre)
                for b in range(BPT):
                    g_ref[par, j, b] = g[:, b * BL:(b + 1) * BL].astype(bf16)
                fire_all(pi, lambda c: pre[(c % 32) * 8:(c % 32) * 8 + 8, (c // 32) * 128:(c // 32) * 128 + 128])
            elif kind == 'mm2':
                j = ph[2]
                if static and t == 0:
                    slabs = [w2_ref[:, (j * SPC + kt) * 128:(j * SPC + kt + 1) * 128] for kt in range(SPC)]
                    for kt in range(SPC):
                        w2p_ref[j * SPC + kt] = _pk(slabs[kt])
                else:
                    slabs = [_upk(w2p_ref[j * SPC + kt]) for kt in range(SPC)]
                gj = jnp.concatenate([_upk(g_w[par, j, b]) for b in range(BPT)], axis=1)
                part = jnp.dot(jnp.concatenate(slabs, axis=1), gj, preferred_element_type=f32)
                state['acc'] = part if j == 0 else state['acc'] + part
                fire_all(pi, lambda c: part[c * 8:c * 8 + 8, 0:128])
            elif kind == 'inv':
                y0 = inv_h(t)
                fire_all(pi, lambda c: y0[c * 8:c * 8 + 8, :])
            elif kind == 'dft':
                su = dft(t)
                fire_all(pi, lambda c: su[c * 8:c * 8 + 8, 0:128])
            elif kind == 'out':
                emit_out(t, slice(0, D))
                for c in out_cp(t):
                    c.start()
                done.add(('out', t))
            elif kind == 'out_rows':
                for rq in range(NRQ):
                    emit_out(t, slice(rq * RQ, (rq + 1) * RQ))
                    for c in out_rows(t, rq):
                        c.start()
            elif kind == 'acc_store':
                acc_ref[par] = state['acc']
            elif kind == 'acc_load':
                state['acc'] = acc_ref[par]

    def mlp(t, j0, j1):
        ph = []
        for j in range(j0, j1):
            if j < NFC:
                ph.append(('mm1', t, j))
            if j > 0:
                ph.append(('mm2', t, j - 1))
        return ph

    def steady(tiles, dfts=(), last=False):
        phases, streams = [], []
        for t in tiles:
            p0 = len(phases)
            phases += [('inv', t + 1)] + mlp(t, 0, NFC + 1)
            for n, td in enumerate(dfts):
                phases.insert(p0 + DFT_POS[n] + n, ('dft', td))
                w = (DFT_POS[0] - 1.9) / len(dfts)
                streams.append(s_kv(td, p0 + 1.5 + n * w, p0 + 1.5 + (n + 1) * w))
            dfts = ()
            end = len(phases) - 0.7
            streams += [s_hln(t + 1, p0 + 1.3, end), s_xs(t + 2, p0 + 1.3, end), s_mac(t + 2, p0 + 1.0, end)]
            phases.append(('out', t))
        if last:
            p0 = len(phases)
            phases += [('inv', 7)] + mlp(6, 0, JS) + [('acc_store', 6)] + mlp(7, 0, JS) + [('acc_store', 7)]
            streams.append(s_hln(7, p0 + 1.3, p0 + 6.0))
        segment(phases, streams)

    wait(G[0])
    prep()
    wait(G[1])
    kv0 = kv_gen(0)
    next(kv0)
    for _ in range(KV0_FIRST):
        step(kv0)
    wait(G[2])
    while step(kv0):
        pass
    dft(0)
    run_all(mac_gen(0))
    wait(G[3])
    run_all(xstats_gen(0))
    inv_h(0)
    wait(G[4])
    run_all(hln_gen(0))
    run_all(w1t_gen(0, 2))
    segment([('mm1', 0, 0), ('mm1', 0, 1)], [s_w1t(2, 3, 0.2, 1.4)])
    wait(G[5])
    segment([('mm1', 0, 2), ('mm1', 0, 3), ('mm1', 0, 4)], [s_w1t(3, 5, 0.0, 1.2), s_w1t(5, 7, 1.0, 2.4)])
    wait(G[6])
    segment([('mm1', 0, 5), ('mm1', 0, 6), ('dft', 1)], [s_kv(1, 0.0, 1.8)])
    wait(G[7])
    segment([('mm2', 0, j) for j in range(4)], [s_xs(1, 0.0, 3.6), s_mac(1, 0.0, 3.6)])
    wait(G[8])
    segment([('inv', 1)] + [('mm2', 0, j) for j in range(4, 7)] + [('out', 0)], [s_hln(1, 1.2, 3.5)])
    wait(G[9])
    segment([('mm1', 1, 0), ('mm1', 1, 1), ('dft', 2), ('dft', 3), ('mm2', 1, 0)],
            [s_kv(2, 0.0, 1.6), s_kv(3, 1.2, 2.7)])
    wait(G[10])
    segment(mlp(1, 2, 4) + [('inv', 2)] + mlp(1, 4, 7) + [('dft', 4), ('mm2', 1, 6), ('out', 1)],
            [s_xs(2, 0.0, 3.4), s_mac(2, 0.0, 3.6), s_kv(4, 4.5, 10.6), s_hln(2, 5.3, 12.2), s_xs(3, 5.3, 12.2),
             s_mac(3, 5.0, 12.3)])
    wait(G[11])
    steady([2], dfts=(5, 6, 7))
    wait(G[12])
    steady([3, 4, 5], last=True)

    def tail(t, carry):
        segment([('acc_load', t)] + mlp(t, JS, NFC + 1) + [('out_rows', t)], [])
        return carry
    jax.lax.fori_loop(NT - 2, NT, tail, 0)

    for t in range(NT - 2):
        wait(out_cp(t))
    for t in range(NT - 2, NT):
        for rq in range(NRQ):
            wait(out_rows(t, rq))


@jax.jit
def pallas_sequential_preLN__ssm_conv_h3__mixer_channel_mlp__prompt_kernel(
    A_q: jax.Array,
    A_k: jax.Array,
    A_v: jax.Array,
    A_shift_k: jax.Array,
    A_ssm_k: jax.Array,
    A_ssm_D: jax.Array,
    B_x: jax.Array,
    B_w1: jax.Array,
    B_b1: jax.Array,
    B_w2: jax.Array,
    B_b2: jax.Array,
):
    del B_x
    ft, gt = _dft_consts()
    any_spec = pl.BlockSpec(memory_space=pl.ANY)
    out_t = pl.pallas_call(
        _kernel,
        out_shape=jax.ShapeDtypeStruct((D, S), bf16),
        in_specs=[any_spec] * 12,
        out_specs=any_spec,
        scratch_shapes=[
            pltpu.VMEM((NT, D, TM), bf16),
            pltpu.VMEM((NT, D, TM), bf16),
            pltpu.VMEM((NT, D, TM), bf16),
            pltpu.VMEM((KS, D), bf16),
            pltpu.VMEM((NT, D, TM), bf16),
            pltpu.VMEM((D,), bf16),
            pltpu.VMEM((D, F), bf16),
            pltpu.VMEM((F // 128, 128), bf16),
            pltpu.VMEM((D, F), bf16),
            pltpu.VMEM((D,), bf16),
            pltpu.VMEM((2, BL // 2, BL), u32),
            pltpu.VMEM((BL, BL), u32),
            pltpu.VMEM((NB, D, BL), bf16),
            pltpu.VMEM((6, D, 128), f32),
            pltpu.VMEM((DP // 128, F, 128), bf16),
            pltpu.VMEM((NB + 1, NP, 6, 8, 128), f32),
            pltpu.VMEM((2, D, 128), f32),
            pltpu.VMEM((BPT, 2, D, 128), bf16),
            pltpu.VMEM((NKV, BPT * D, 128), bf16),
            pltpu.VMEM((2, BPT, D, BL), f32),
            pltpu.VMEM((2, BPT, DP, BL), bf16),
            pltpu.VMEM((2, D, TM), f32),
            pltpu.VMEM((BPT, 2, 8, 128), f32),
            pltpu.VMEM((F // 128, D // 2, 128), u32),
            pltpu.VMEM((2, NFC, BPT, FC, BL), bf16),
            pltpu.SemaphoreType.DMA((NSEM,)),
        ],
        compiler_params=pltpu.CompilerParams(vmem_limit_bytes=110 * 1024 * 1024),
    )(A_q[0].T, A_k[0].T, A_v[0].T, A_shift_k.T, A_ssm_k, A_ssm_D, B_w1,
      B_b1.reshape(F // 128, 128), B_w2.T, B_b2, ft, gt)
    return out_t.T[None]
```
